```python
import jax
import jax.numpy as jnp

def _softmax(x, axis=-1):
    return jax.nn.softmax(x, axis=axis)

def _gelu(x):
    return jax.nn.gelu(x, approximate=True)

def _silu(x):
    return jax.nn.silu(x)

def _sigmoid(x):
    return jax.nn.sigmoid(x)

def _layernorm(x, axis=-1, eps=1e-05):
    m = jnp.mean(x, axis=axis, keepdims=True)
    v = jnp.var(x, axis=axis, keepdims=True)
    return (x - m) / jnp.sqrt(v + eps)

def _scatter_add(tgt, idx, src, axis=0):
    return tgt.at[idx].add(src)

def _segment_sum(src, seg, n):
    return jax.ops.segment_sum(src, seg, n)

class _Rng:

    def __init__(self, key):
        self._k = key

    def _next(self):
        self._k, sub = jax.random.split(self._k)
        return sub

    def normal(self, shape):
        return jax.random.normal(self._next(), shape, dtype=jnp.bfloat16)

    def randint(self, lo, hi, shape):
        return jax.random.randint(self._next(), shape, lo, hi, dtype=jnp.int32)

    def uniform(self, shape, lo=0.0, hi=1.0):
        return jax.random.uniform(self._next(), shape, jnp.bfloat16, lo, hi)

    def permutation(self, n):
        return jax.random.permutation(self._next(), n)
kernel_name = 'standalone__autoregressive_conv_wavernn__speech'

def setup_inputs():
    _rng = _Rng(jax.random.key(int.from_bytes(__import__("os").urandom(4), "little")))
    _w = lambda a: (lambda t: t.astype(jnp.bfloat16) if jnp.issubdtype(t.dtype, jnp.floating) else t)(jnp.asarray(a))
    B, T, D, K = (2, 16000, 256, 31)
    return {'x': _w((lambda *s: _rng.normal(s) * 0.05)(B, T, D)), 'w': _w((lambda *s: _rng.normal(s) * 0.05)(K, D, 2 * D))}

def reference(x, w):
    B, T, D = x.shape
    K = w.shape[0]
    dil = 2
    pad = (K - 1) * dil
    xp = jnp.pad(x, ((0, 0), (pad, 0), (0, 0)))
    h = jnp.einsum('btd,de->bte', xp[:, 0:T, :], w[0])
    for i in range(1, K):
        h = h + jnp.einsum('btd,de->bte', xp[:, i * dil:i * dil + T, :], w[i])
    f, g = (h[..., :D].copy(), h[..., D:].copy())
    return jnp.tanh(f) * _sigmoid(g)
```

```python
import jax
import jax.numpy as jnp
import jax.experimental.pallas as pl
import jax.experimental.pallas.tpu as pltpu

DIL = 2


@jax.jit
def pallas_standalone__autoregressive_conv_wavernn__speech_kernel(x, w):
    B, T, D = x.shape
    K = w.shape[0]
    pad = (K - 1) * DIL
    TT = 800
    assert T % TT == 0
    HALO = 64
    xp = jnp.pad(x, ((0, 0), (HALO, 0), (0, 0)))

    def kernel(x_ref, w_ref, o_ref):
        t = pl.program_id(1)
        base = pl.multiple_of(t * TT, TT)
        xs = x_ref[pl.ds(base, TT + HALO), :].astype(jnp.float32)
        acc = jnp.zeros((TT, 2 * D), jnp.float32)
        for k in range(K):
            off = HALO - pad + k * DIL
            acc += jnp.dot(xs[off:off + TT].astype(jnp.bfloat16), w_ref[k],
                           preferred_element_type=jnp.float32)
        f = acc[:, :D]
        g = acc[:, D:]
        o_ref[...] = (jnp.tanh(f) * jax.nn.sigmoid(g)).astype(o_ref.dtype)

    return pl.pallas_call(
        kernel,
        grid=(B, T // TT),
        in_specs=[
            pl.BlockSpec((None, T + HALO, D), lambda b, t: (b, 0, 0)),
            pl.BlockSpec((K, D, 2 * D), lambda b, t: (0, 0, 0)),
        ],
        out_specs=pl.BlockSpec((None, TT, D), lambda b, t: (b, t, 0)),
        out_shape=jax.ShapeDtypeStruct((B, T, D), x.dtype),
        compiler_params=pltpu.CompilerParams(
            dimension_semantics=("parallel", "arbitrary"),
            vmem_limit_bytes=100 * 1024 * 1024),
    )(xp, w)
```

```python
import functools
import numpy as np
import jax
import jax.numpy as jnp
from jax import lax
import jax.experimental.pallas as pl
import jax.experimental.pallas.tpu as pltpu

N = 128
L = 96
HIST = N - L
NF = N // 2
bf16 = jnp.bfloat16
u32 = jnp.uint32
f32 = jnp.float32


def _consts(K):
    th = 2 * np.pi * (np.arange(NF) + 0.5) / N
    n = np.arange(N)
    F = np.concatenate([np.cos(th[:, None] * n), -np.sin(th[:, None] * n)], 0)
    m = np.arange(L) + HIST
    G = np.zeros((L, NF, 2)); G[:, :, 0] = np.cos(th[None] * m[:, None]) * 2 / N
    G[:, :, 1] = -np.sin(th[None] * m[:, None]) * 2 / N
    G = G.reshape(L, N)
    j = (K - 1) - np.arange(K)
    C = np.zeros((N, 32))
    C[:NF, :K] = np.cos(th[:, None] * j); C[NF:, :K] = -np.sin(th[:, None] * j)
    Cb = np.zeros((2, 4 * N, 128))
    for g in range(4):
        Cb[0, g * N:(g + 1) * N, g * 32:(g + 1) * 32] = C
    Cb[1] = 0.5 * Cb[0]
    return (np.asarray(F, dtype=bf16), np.asarray(G, dtype=bf16), np.asarray(Cb, dtype=bf16))


def _unpack(x):
    return [pltpu.unpack_elementwise(x, index=i, packed_dtype=bf16, unpacked_dtype=f32) for i in range(2)]


def _pack(a, b):
    return pltpu.pack_elementwise([a, b], packed_dtype=bf16)


def make(B, T, D, K, NB=56, stages=(1, 1, 1, 1), u1=1, u2=1, u3=1, uw=1, fuse=True, OCH=28):
    HOP = 2 * L
    nblk = -(-T // HOP)
    NQ = B * nblk
    assert NQ % NB == 0
    NS = NQ // NB
    BSTR = nblk * HOP
    HEAD = 2 * HIST
    XROWS = NQ * HOP + HEAD
    D2 = 2 * D
    ET = D2 // 128
    DT = D // 128
    H = D // 2
    HP = H + 4
    P = NB + 4 if NB % 8 == 0 else NB
    PY = 2 * NB + 4
    assert NF * PY >= 32 * HP
    NOC = NQ // OCH
    assert nblk % OCH == 0

    def kernel(x_hbm, w_hbm, F_ref, G_ref, C_ref, o_hbm, xs, wv, W3, Xh, Yh, ost, sems, osems):
        wcps = [pltpu.make_async_copy(w_hbm.at[:, pl.ds(e * 128, 128)], wv.at[e], sems.at[e]) for e in range(ET)]
        for c in wcps:
            c.start()
        xcps = [pltpu.make_async_copy(x_hbm.at[b, :, pl.ds(d * 128, 128)], xs.at[d, pl.ds(b * BSTR + HEAD, T)],
                                      sems.at[ET + b * DT + d])
                for b in range(B) for d in range(DT)]
        for c in xcps:
            c.start()
        for d in range(DT):
            xs[d, pl.ds(0, HEAD), :] = jnp.zeros((HEAD, 128), bf16)
            for b in range(B):
                xs[d, pl.ds(b * BSTR + HEAD + T, BSTR - T), :] = jnp.zeros((BSTR - T, 128), bf16)

        for e in range(ET):
            wcps[e].wait()
            def wcopy(k, carry):
                wd = pltpu.bitcast(wv[e, pl.ds(pl.multiple_of(k * D, D), D), :], u32)
                Yh[e, pl.ds(pl.multiple_of(k * HP, 4), H), :] = wd
                return carry
            lax.fori_loop(0, K, wcopy, 0)
            for k in range(K, 32):
                Yh[e, pl.ds(k * HP, H), :] = jnp.zeros((H, 128), u32)
            if stages[0]:
                def wbody(jg, carry):
                    cols = []
                    for t in range(4):
                        parts = []
                        for jj in range(2):
                            j = (jg * 4 + t) * 2 + jj
                            parts += _unpack(Yh[e, pl.ds(j, 32, stride=HP), :])
                        cols.append(jnp.concatenate(parts, 0).astype(bf16))
                    rhs = jnp.concatenate(cols, 1)
                    res = jnp.dot(C_ref[e // DT], rhs, preferred_element_type=f32)
                    for t in range(4):
                        r = res[:, t * 128:(t + 1) * 128]
                        for jj in range(2):
                            j = (jg * 4 + t) * 2 + jj
                            m = []
                            for g in (2 * jj, 2 * jj + 1):
                                vr = r[g * N:g * N + NF]
                                vi = r[g * N + NF:(g + 1) * N]
                                m.append((vr, vi - vr, vi + vr))
                            for c in range(3):
                                W3[e, pl.ds(c * NF * HP + j, NF, stride=HP), :] = _pack(m[0][c], m[1][c])
                    return carry
                lax.fori_loop(0, H // 8, wbody, 0, unroll=uw)

        for c in xcps:
            c.wait()

        def s1(q, il):
            r0 = pl.multiple_of(q * HOP, HOP)
            cols = []
            for d in range(DT):
                xw = pltpu.bitcast(xs[d, pl.ds(r0, 2 * N), :], u32)
                cols.append([v.astype(bf16) for v in _unpack(xw)])
            rhs = jnp.concatenate([cols[d][p] for d in range(DT) for p in range(2)], 1)
            res = jnp.dot(F_ref[...], rhs, preferred_element_type=f32)
            for d in range(DT):
                ev = res[:, (2 * d) * 128:(2 * d + 1) * 128]
                od = res[:, (2 * d + 1) * 128:(2 * d + 2) * 128]
                m = [(v[:NF] + v[NF:], v[:NF], v[NF:]) for v in (ev, od)]
                for c in range(3):
                    Xh[d, pl.ds(c * NF * P + il, NF, stride=P), :] = _pack(m[0][c], m[1][c])

        def s2(f, carry):
            k = []
            for c in range(3):
                r = (c * NF + f) * P
                lhs = jnp.concatenate([pltpu.bitcast(Xh[d, pl.ds(r, NB), :], bf16) for d in range(DT)], 1)
                rw = (c * NF + f) * HP
                wf = jnp.concatenate([pltpu.bitcast(W3[e, pl.ds(rw, H), :], bf16) for e in range(ET)], 1)
                k.append(jnp.dot(lhs, wf, preferred_element_type=f32))
            p = _pack(k[0] - k[2], k[0] + k[1])
            for e in range(ET):
                Yh[e, pl.ds(f * PY, 2 * NB), :] = p[:, e * 128:(e + 1) * 128]
            return carry

        def s3(q, il):
            z = []
            for p in range(2):
                yw = jnp.concatenate([pltpu.bitcast(Yh[e, pl.ds(2 * il + p, NF, stride=PY), :], bf16) for e in range(ET)], 1)
                z.append(jnp.dot(G_ref[...], yw, preferred_element_type=f32))
            outs = []
            for p in range(2):
                tf = jnp.tanh(z[p][:, :D]) * 0.5
                outs.append(tf + tf * jnp.tanh(z[p][:, D:]))
            o = pltpu.bitcast(_pack(outs[0], outs[1]), bf16)
            for d in range(DT):
                ost[d, pl.ds(pl.multiple_of(q * HOP, HOP), HOP), :] = o[:, d * 128:(d + 1) * 128]

        ocps = []

        def out_chunk(ch):
            b, i0 = divmod(ch * OCH, nblk)
            t0 = i0 * HOP
            n = min(OCH * HOP, T - t0)
            for d in range(DT):
                cp = pltpu.make_async_copy(ost.at[d, pl.ds(b * BSTR + t0, n)],
                                           o_hbm.at[b, pl.ds(t0, n), pl.ds(d * 128, 128)], osems.at[ch * DT + d])
                cp.start()
                ocps.append(cp)

        def loop1(s):
            def body(il, carry):
                s1(s * NB + il, il)
                return carry
            lax.fori_loop(0, NB, body, 0, unroll=u1)

        def loop3(s, with_s1):
            assert NB % OCH == 0
            for h in range(NB // OCH):
                def body(i, carry):
                    il = h * OCH + i
                    s3(s * NB + il, il)
                    if with_s1:
                        s1((s + 1) * NB + il, il)
                    return carry
                lax.fori_loop(0, OCH, body, 0, unroll=u3)
                out_chunk((s * NB) // OCH + h)

        if stages[1]:
            loop1(0)
        for s in range(NS):
            if stages[2]:
                lax.fori_loop(0, NF, s2, 0, unroll=u2)
            nxt = s + 1 < NS
            if stages[3]:
                loop3(s, fuse and nxt and stages[1])
            if nxt and stages[1] and not (fuse and stages[3]):
                loop1(s + 1)
        for c in ocps:
            c.wait()

    Fm, Gm, Cm = _consts(K)

    def fn(x, w):
        return pl.pallas_call(
            kernel,
            in_specs=[pl.BlockSpec(memory_space=pl.ANY), pl.BlockSpec(memory_space=pl.ANY),
                      pl.BlockSpec(memory_space=pltpu.VMEM), pl.BlockSpec(memory_space=pltpu.VMEM),
                      pl.BlockSpec(memory_space=pltpu.VMEM)],
            out_specs=pl.BlockSpec(memory_space=pl.ANY),
            out_shape=jax.ShapeDtypeStruct((B, T, D), x.dtype),
            scratch_shapes=[
                pltpu.VMEM((DT, XROWS, 128), bf16),
                pltpu.VMEM((ET, K * D, 128), bf16),
                pltpu.VMEM((ET, 3 * NF * HP, 128), u32),
                pltpu.VMEM((DT, 3 * NF * P, 128), u32),
                pltpu.VMEM((ET, NF * PY, 128), u32),
                pltpu.VMEM((DT, NQ * HOP, 128), bf16),
                pltpu.SemaphoreType.DMA((ET + B * DT,)),
                pltpu.SemaphoreType.DMA((NOC * DT,)),
            ],
            compiler_params=pltpu.CompilerParams(vmem_limit_bytes=127 * 1024 * 1024),
        )(x, w.reshape(K * D, D2), Fm, Gm, Cm)
    return fn


@jax.jit
def pallas_standalone__autoregressive_conv_wavernn__speech_kernel(x, w):
    B, T, D = x.shape
    K = w.shape[0]
    return make(B, T, D, K, )(x, w)
```

```python
import functools
import numpy as np
import jax
import jax.numpy as jnp
from jax import lax
import jax.experimental.pallas as pl
import jax.experimental.pallas.tpu as pltpu

N = 128
L = 96
HIST = N - L
NF = N // 2
bf16 = jnp.bfloat16
u32 = jnp.uint32
f32 = jnp.float32


def _consts(K):
    th = 2 * np.pi * (np.arange(NF) + 0.5) / N
    n = np.arange(N)
    F = np.concatenate([np.cos(th[:, None] * n), -np.sin(th[:, None] * n)], 0)
    m = np.arange(L) + HIST
    G = np.zeros((L, NF, 2)); G[:, :, 0] = np.cos(th[None] * m[:, None]) * 2 / N
    G[:, :, 1] = -np.sin(th[None] * m[:, None]) * 2 / N
    G = G.reshape(L, N)
    j = (K - 1) - np.arange(K)
    C = np.zeros((N, 32))
    C[:NF, :K] = np.cos(th[:, None] * j); C[NF:, :K] = -np.sin(th[:, None] * j)
    Cb = np.zeros((2, 4 * N, 128))
    for jj in range(2):
        for dd in range(2):
            g = 2 * jj + dd
            Cb[0, g * N:(g + 1) * N, jj * 64 + dd:(jj + 1) * 64:2] = C
    Cb = Cb.reshape(2, 2, 2, 2, 8, 8, 128).transpose(0, 1, 4, 2, 3, 5, 6).reshape(2, 4 * N, 128)
    Cb[1] = 0.5 * Cb[0]
    return (np.asarray(F, dtype=bf16), np.asarray(G, dtype=bf16), np.asarray(Cb, dtype=bf16))


def _unpack(x):
    return [pltpu.unpack_elementwise(x, index=i, packed_dtype=bf16, unpacked_dtype=f32) for i in range(2)]


def _pack(a, b):
    return pltpu.pack_elementwise([a, b], packed_dtype=bf16)


def make(B, T, D, K, NB=56, stages=(1, 1, 1, 1), u1=7, u2=4, u3=7, uw=2, WCH=(4, 4, 4, 4), OCB=7, nodma=0, LCS=(7,) * 8, w0=16):
    HOP = 2 * L
    nblk = -(-T // HOP)
    NQ = B * nblk
    assert NQ % NB == 0
    NS = NQ // NB
    BSTR = nblk * HOP
    HEAD = 2 * HIST
    XROWS = NQ * HOP + HEAD
    D2 = 2 * D
    ET = D2 // 128
    DT = D // 128
    H = D // 2
    HP = H + 4
    P = NB + 4 if NB % 8 == 0 else NB
    PY = 2 * NB + 4
    assert nblk % OCB == 0 and NB % u3 == 0 and u3 % OCB == 0
    CPB = nblk // OCB
    CH = OCB * HOP
    CHL = T - (CPB - 1) * CH
    assert sum(LCS) == NB
    WC = len(WCH)
    assert sum(WCH) * 16 == D
    WOFF = [sum(WCH[:c]) for c in range(WC)]

    xpieces = []
    for b in range(B):
        cuts = sorted({0, T} | {s * NB * HOP - b * BSTR for s in range(1, NS) if 0 < s * NB * HOP - b * BSTR < T})
        for t0, t1 in zip(cuts[:-1], cuts[1:]):
            first = (b * BSTR + HEAD + t0 - 2 * N) // HOP + 1
            xpieces.append((max(first, 0) // NB, b, t0, t1 - t0))

    def kernel(x_hbm, w_hbm, F_hbm, G_hbm, C_hbm, o_hbm, xs, wv, W3, Xh, Yh, ost, F_ref, G_ref, C_ref, wsem, xsem, osem, csem, lsem):
        wcps = [pltpu.make_async_copy(w_hbm.at[:, pl.ds(WOFF[c] * 16, WCH[c] * 16), :],
                                      wv.at[pl.ds(0, K), pl.ds(WOFF[c] * 16, WCH[c] * 16), :], wsem.at[c])
                for c in range(WC)]
        xcps = [[pltpu.make_async_copy(x_hbm.at[b, pl.ds(t0, n), pl.ds(d * 128, 128)],
                                       xs.at[d, pl.ds(b * BSTR + HEAD + t0, n)], xsem.at[i * DT + d])
                 for d in range(DT)] for i, (_, b, t0, n) in enumerate(xpieces)]
        ccps = [pltpu.make_async_copy(a, b_, csem.at[i]) for i, (a, b_) in enumerate(((C_hbm, C_ref), (F_hbm, F_ref), (G_hbm, G_ref)))]
        if nodma & 1:
            class _N:
                def start(self): pass
                def wait(self): pass
            ccps = [_N()] * 3
            wcps = [_N()] * WC
            xcps = [[_N()] * DT] * len(xpieces)
        ccps[0].start()
        wcps[0].start()
        if WC > 1:
            wcps[1].start()
        ccps[1].start()
        ccps[2].start()
        for d in range(DT):
            xs[d, pl.ds(0, HEAD), :] = jnp.zeros((HEAD, 128), bf16)
            for b in range(B):
                xs[d, pl.ds(b * BSTR + HEAD + T, BSTR - T), :] = jnp.zeros((BSTR - T, 128), bf16)
        for k in range(K, 32):
            wv[k] = jnp.zeros((D, D2), bf16)

        xi = [0]

        def start_x(upto_s):
            while xi[0] < len(xpieces) and xpieces[xi[0]][0] <= upto_s:
                for c in xcps[xi[0]]:
                    c.start()
                xi[0] += 1

        def wait_x(s):
            for i, pc in enumerate(xpieces):
                if pc[0] == s:
                    for c in xcps[i]:
                        c.wait()

        for c in range(WC):
            wcps[c].wait()
            if c == 0:
                ccps[0].wait()
            if c + 2 < WC:
                wcps[c + 2].start()
            if c + 2 == WC or WC == 1:
                start_x(0)
            if c == WC - 1:
                start_x(NS)
            if stages[0]:
                def wbody(it, carry):
                    jg = WOFF[c] + it
                    for e in range(ET):
                        wd = pltpu.bitcast(wv[:, pl.ds(pl.multiple_of(jg * 16, 16), 16), e * 128:(e + 1) * 128], u32)
                        wd = jnp.swapaxes(wd, 0, 1)
                        rhs = jnp.concatenate([pltpu.bitcast(wd[2 * t:2 * t + 2].reshape(64, 128), bf16) for t in range(4)], 1)
                        res = jnp.dot(C_ref[e // DT], rhs, preferred_element_type=f32)
                        for jj in range(2):
                            for fo in range(8):
                                r0 = (jj * 8 + fo) * 32
                                for t in range(4):
                                    m = []
                                    for dd in range(2):
                                        vr = res[r0 + dd * 16:r0 + dd * 16 + 8, t * 128:(t + 1) * 128]
                                        vi = res[r0 + dd * 16 + 8:r0 + dd * 16 + 16, t * 128:(t + 1) * 128]
                                        m.append((vr, vi - vr, vi + vr))
                                    for cc in range(3):
                                        W3[e, pl.ds((cc * NF + fo * 8) * HP + jg * 8 + 2 * t + jj, 8, stride=HP), :] = _pack(m[0][cc], m[1][cc])
                    return carry
                lax.fori_loop(0, WCH[c], wbody, 0, unroll=min(uw, WCH[c]))

        def s1(q, il):
            r0 = pl.multiple_of(q * HOP, HOP)
            cols = []
            for d in range(DT):
                xw = pltpu.bitcast(xs[d, pl.ds(r0, 2 * N), :], u32)
                cols.append([v.astype(bf16) for v in _unpack(xw)])
            rhs = jnp.concatenate([cols[d][p] for d in range(DT) for p in range(2)], 1)
            res = jnp.dot(F_ref[...], rhs, preferred_element_type=f32)
            for d in range(DT):
                ev = res[:, (2 * d) * 128:(2 * d + 1) * 128]
                od = res[:, (2 * d + 1) * 128:(2 * d + 2) * 128]
                m = [(v[:NF] + v[NF:], v[:NF], v[NF:]) for v in (ev, od)]
                for c in range(3):
                    Xh[d, pl.ds(c * NF * P + il, NF, stride=P), :] = _pack(m[0][c], m[1][c])

        def s2(f, carry):
            k = []
            for c in range(3):
                r = (c * NF + f) * P
                lhs = jnp.concatenate([pltpu.bitcast(Xh[d, pl.ds(r, NB), :], bf16) for d in range(DT)], 1)
                rw = (c * NF + f) * HP
                wf = jnp.concatenate([pltpu.bitcast(W3[e, pl.ds(rw, H), :], bf16) for e in range(ET)], 1)
                k.append(jnp.dot(lhs, wf, preferred_element_type=f32))
            p = _pack(k[0] - k[2], k[0] + k[1])
            for e in range(ET):
                Yh[e, pl.ds(f * PY, 2 * NB), :] = p[:, e * 128:(e + 1) * 128]
            return carry

        def s3(q, il):
            z = []
            for p in range(2):
                yw = jnp.concatenate([pltpu.bitcast(Yh[e, pl.ds(2 * il + p, NF, stride=PY), :], bf16) for e in range(ET)], 1)
                z.append(jnp.dot(G_ref[...], yw, preferred_element_type=f32))
            outs = []
            for p in range(2):
                tf = jnp.tanh(z[p][:, :D]) * 0.5
                outs.append(tf + tf * jnp.tanh(z[p][:, D:]))
            o = pltpu.bitcast(_pack(outs[0], outs[1]), bf16)
            for d in range(DT):
                ost[d, pl.ds(pl.multiple_of(q * HOP, HOP), HOP), :] = o[:, d * 128:(d + 1) * 128]

        def out_copy(ch, d):
            b = ch // CPB
            t0 = pl.multiple_of((ch % CPB) * CH, CH)
            n = jnp.where((ch % CPB) == CPB - 1, CHL, CH) if not isinstance(ch, int) else (CHL if ch % CPB == CPB - 1 else CH)
            if not isinstance(ch, int):
                n = pl.multiple_of(n, 64)
            return pltpu.make_async_copy(ost.at[d, pl.ds(pl.multiple_of(b * BSTR + t0, 64), n)],
                                         o_hbm.at[b, pl.ds(t0, n), pl.ds(d * 128, 128)], osem.at[ch * DT + d])

        def out_do(ch, what):
            if nodma & 2:
                return
            for d in range(DT):
                getattr(out_copy(ch, d), what)()

        lcps = []

        def last_copy(q0, nq):
            if nodma & 2:
                return
            b, i0 = divmod(q0, nblk)
            t0 = i0 * HOP
            n = min(nq * HOP, T - t0)
            for d in range(DT):
                cp = pltpu.make_async_copy(ost.at[d, pl.ds(q0 * HOP, n)], o_hbm.at[b, pl.ds(t0, n), pl.ds(d * 128, 128)],
                                           lsem.at[len(lcps)])
                cp.start()
                lcps.append(cp)

        def loop1(s):
            def body(il, carry):
                s1(s * NB + il, il)
                return carry
            lax.fori_loop(0, NB, body, 0, unroll=u1)

        def loop3(s, with_s1):
            def body(i, carry):
                for t in range(u3):
                    il = i * u3 + t
                    if stages[3]:
                        s3(s * NB + il, il)
                    if with_s1 and stages[1]:
                        s1((s + 1) * NB + il, il)
                    if stages[3] and (t + 1) % OCB == 0:
                        out_do(s * (NB // OCB) + i * (u3 // OCB) + t // OCB, 'start')
                return carry
            lax.fori_loop(0, NB // u3, body, 0)

        ccps[1].wait()
        ccps[2].wait()
        wait_x(0)
        if stages[1]:
            loop1(0)

        def sbody(s, carry):
            if stages[2]:
                lax.fori_loop(0, NF, s2, 0, unroll=u2)

            for ss in range(NS - 1):
                @pl.when(s == ss)
                def _():
                    wait_x(ss + 1)

            @pl.when(s < NS - 1)
            def _():
                loop3(s, True)
            return carry
        lax.fori_loop(0, NS, sbody, 0)

        il = 0
        for n in LCS:
            for t in range(n):
                if stages[3]:
                    s3((NS - 1) * NB + il + t, il + t)
            last_copy((NS - 1) * NB + il, n)
            il += n

        if stages[3]:
            def owait(ch, carry):
                out_do(ch, 'wait')
                return carry
            lax.fori_loop(0, (NS - 1) * (NB // OCB), owait, 0)
            for cp in lcps:
                cp.wait()

    Fm, Gm, Cm = _consts(K)

    def fn(x, w):
        return pl.pallas_call(
            kernel,
            in_specs=[pl.BlockSpec(memory_space=pl.ANY)] * 5,
            out_specs=pl.BlockSpec(memory_space=pl.ANY),
            out_shape=jax.ShapeDtypeStruct((B, T, D), x.dtype),
            scratch_shapes=[
                pltpu.VMEM((DT, XROWS, 128), bf16),
                pltpu.VMEM((32, D, D2), bf16),
                pltpu.VMEM((ET, 3 * NF * HP, 128), u32),
                pltpu.VMEM((DT, 3 * NF * P, 128), u32),
                pltpu.VMEM((ET, NF * PY, 128), u32),
                pltpu.VMEM((DT, NQ * HOP, 128), bf16),
                pltpu.VMEM(Fm.shape, bf16),
                pltpu.VMEM(Gm.shape, bf16),
                pltpu.VMEM(Cm.shape, bf16),
                pltpu.SemaphoreType.DMA((WC,)),
                pltpu.SemaphoreType.DMA((len(xpieces) * DT,)),
                pltpu.SemaphoreType.DMA((B * CPB * DT,)),
                pltpu.SemaphoreType.DMA((3,)),
                pltpu.SemaphoreType.DMA((len(LCS) * DT,)),
            ],
            compiler_params=pltpu.CompilerParams(vmem_limit_bytes=127 * 1024 * 1024),
        )(x, w, Fm, Gm, Cm)
    return fn


@jax.jit
def pallas_standalone__autoregressive_conv_wavernn__speech_kernel(x, w):
    B, T, D = x.shape
    K = w.shape[0]
    return make(B, T, D, K, u2=16,u3=28,u1=28,OCB=14,LCS=(7,)*7+(4,2,1),WCH=(2,4,4,6),uw=2)(x, w)
```

```python
import math
import numpy as np
import jax
import jax.numpy as jnp
from jax import lax
import jax.experimental.pallas as pl
import jax.experimental.pallas.tpu as pltpu

N = 128
L = 96
HIST = N - L
NF = N // 2
bf16 = jnp.bfloat16
u32 = jnp.uint32
f32 = jnp.float32


def _consts(K):
    th = np.pi * (4 * np.arange(NF) + 1) / N
    n = np.arange(N)
    F = np.concatenate([np.cos(th[:, None] * n), np.sin(th[:, None] * n)], 0)
    m = np.arange(L) + HIST
    G = np.zeros((L, NF, 2)); G[:, :, 0] = np.cos(th[None] * m[:, None]) * 2 / N
    G[:, :, 1] = np.sin(th[None] * m[:, None]) * 2 / N
    G = G.reshape(L, N)
    j = (K - 1) - np.arange(K)
    C = np.zeros((N, 32))
    C[:NF, :K] = np.cos(th[:, None] * j); C[NF:, :K] = np.sin(th[:, None] * j)
    Cb = np.zeros((2, 4 * N, 128))
    for jj in range(2):
        for dd in range(2):
            g = 2 * jj + dd
            Cb[0, g * N:(g + 1) * N, jj * 64 + dd:(jj + 1) * 64:2] = C
    Cb = Cb.reshape(2, 2, 2, 2, 8, 8, 128).transpose(0, 1, 4, 2, 3, 5, 6).reshape(2, 4 * N, 128)
    Cb[1] = 0.5 * Cb[0]
    return np.asarray(np.concatenate([F, Cb[0], Cb[1], G], 0), dtype=bf16)


def _unpack(x):
    return [pltpu.unpack_elementwise(x, index=i, packed_dtype=bf16, unpacked_dtype=f32) for i in range(2)]


def _pack(a, b):
    return pltpu.pack_elementwise([a, b], packed_dtype=bf16)


def _cmul(re, im, w):
    c, s = w.real, w.imag
    eps = 1e-12
    def close(a, b): return abs(a - b) < eps
    if close(c, 1) and close(s, 0): return re, im
    if close(c, -1) and close(s, 0): return -re, -im
    if close(c, 0) and close(s, 1): return -im, re
    if close(c, 0) and close(s, -1): return im, -re
    if close(abs(c), abs(s)):
        a = c
        if close(s, c):
            return (re - im) * a, (re + im) * a
        else:
            return (re + im) * a, (im - re) * a
    return re * c - im * s, re * s + im * c

def _fft(xs, sign=-1):
    n = len(xs)
    if n == 1: return xs
    if n == 2:
        (a, b), (c, d) = xs
        return [(a + c, b + d), (a - c, b - d)]
    if n == 4:
        (a0, b0), (a1, b1), (a2, b2), (a3, b3) = xs
        s0r, s0i, d0r, d0i = a0 + a2, b0 + b2, a0 - a2, b0 - b2
        s1r, s1i, d1r, d1i = a1 + a3, b1 + b3, a1 - a3, b1 - b3
        if sign < 0:
            return [(s0r + s1r, s0i + s1i), (d0r + d1i, d0i - d1r), (s0r - s1r, s0i - s1i), (d0r - d1i, d0i + d1r)]
        return [(s0r + s1r, s0i + s1i), (d0r - d1i, d0i + d1r), (s0r - s1r, s0i - s1i), (d0r + d1i, d0i - d1r)]
    ev = _fft(xs[0::2], sign); od = _fft(xs[1::2], sign)
    out = [None] * n
    for k in range(n // 2):
        w = complex(math.cos(2 * math.pi * k / n), sign * math.sin(2 * math.pi * k / n))
        if abs(w.real) < 1e-12 and abs(w.imag - sign) < 1e-12:
            r, i_ = od[k]
            if sign < 0:
                out[k] = (ev[k][0] + i_, ev[k][1] - r); out[k + n // 2] = (ev[k][0] - i_, ev[k][1] + r)
            else:
                out[k] = (ev[k][0] - i_, ev[k][1] + r); out[k + n // 2] = (ev[k][0] + i_, ev[k][1] - r)
            continue
        tr, ti = _cmul(od[k][0], od[k][1], w)
        out[k] = (ev[k][0] + tr, ev[k][1] + ti)
        out[k + n // 2] = (ev[k][0] - tr, ev[k][1] - ti)
    return out

def _rot(ph):
    return complex(math.cos(ph), math.sin(ph))


def _fwd128(loadw, tst, tld, emit, gate):
    for n2 in range(8):
        for p in range(2):
            g = gate()
            col = []
            for n1 in range(8):
                a = loadw(8 * n1 + n2, p, g); b = loadw(8 * n1 + n2 + 64, p, g)
                col.append(_cmul(a, b, _rot(math.pi * 8 * n1 / 128)))
            o = _fft(col, +1)
            for g1 in range(8):
                r, i_ = _cmul(o[g1][0], o[g1][1], _rot(2 * math.pi * g1 * n2 / 64 + math.pi * n2 / 128))
                tst(((p * 8 + g1) * 8 + n2) * 2, r); tst(((p * 8 + g1) * 8 + n2) * 2 + 1, i_)
            yield
    for g1 in range(8):
        for p in range(2):
            g = gate()
            o = _fft([(tld(((p * 8 + g1) * 8 + n2) * 2, g), tld(((p * 8 + g1) * 8 + n2) * 2 + 1, g)) for n2 in range(8)], +1)
            if p == 0:
                o0 = o
            else:
                for g2 in range(8):
                    emit(g1 + 8 * g2, [o0[g2], o[g2]])
            yield


def make(B, T, D, K, NB=56, u1=28, u2=32, u3=14, uw=2, nodma=0, LCS=(7, 4, 2, 1), XAT=4, WSL=8,
         GT=(0, 2), GOFF=0.0, flags=None, XMV='v', XG=1, XSCH=None):
    HOP = 2 * L
    nblk = -(-T // HOP)
    NQ = B * nblk
    assert NQ % NB == 0 and NB % 8 == 0
    NS = NQ // NB
    BSTR = nblk * HOP
    HEAD = 2 * HIST
    XROWS = NQ * HOP + HEAD
    D2 = 2 * D
    ET = D2 // 128
    DT = D // 128
    H = D // 2
    HP = H + 1
    P = NB + 1 if NB % 8 == 0 else NB
    PY = 2 * NB + 1
    XP = L + 4
    OCB = u3
    assert nblk % OCB == 0 and NB % u3 == 0
    CPB = nblk // OCB
    CH = OCB * HOP
    CHL = T - (CPB - 1) * CH
    NCS = NB // OCB
    WC = D // 16
    NWI = WC // uw
    WSCH = [list(range(uw))]
    nxt = uw
    while nxt < WC:
        i = len(WSCH) - 1
        hi = min(nxt + uw + 1, WC, i * uw + WSL)
        WSCH.append(list(range(nxt, hi)))
        nxt = hi
    nl = NB - sum(LCS)
    assert nl % u3 == 0 and sum(LCS) == u3
    NU = (NB // 8) * DT
    NI2 = NF // u2
    assert NU % NI2 == 0
    FU = NU // NI2

    XB = 8
    xpieces = []
    for j in range(NQ // XB):
        lo, hi = j * XB * HOP + HEAD, (j + 1) * XB * HOP + HEAD
        parts = []
        for b in range(B):
            r0, r1 = max(lo, b * BSTR + HEAD), min(hi, b * BSTR + HEAD + T)
            if r1 > r0:
                parts.append((b, r0 - b * BSTR - HEAD, r1 - r0))
        xpieces.append(parts)
    PPS = NB // XB
    if XSCH is None:
        XSCH = [[], [0], [1], [2], [3, 4], [5, 6], [7, 8], [9, 10]]
    xlate = [j for j in range(2 * PPS) if not any(j in z for z in XSCH)]
    nxs = sum(len(p) for p in xpieces)

    consts = _consts(K)
    RF, RC, RG = 0, N, N + 8 * N

    def kernel(x_hbm, w_hbm, c_hbm, z_ref, o_hbm, xs, wv, W3, Xh, Xn, Yh, ost, cv, xu, TT, wsem, xsem, osem, lsem, csem, msem):
        def wcp(c):
            r = c * 16 if isinstance(c, int) else pl.multiple_of(c * 16, 16)
            return pltpu.make_async_copy(w_hbm.at[:, pl.ds(r, 16), :], wv.at[c % WSL, pl.ds(0, K)], wsem.at[c % WSL])

        xcps = []
        for parts in xpieces:
            xcps.append([pltpu.make_async_copy(x_hbm.at[b, pl.ds(t0, n), :], xs.at[pl.ds(b * BSTR + HEAD + t0, n), :],
                                               xsem.at[sum(map(len, xcps)) + i]) for i, (b, t0, n) in enumerate(parts)])
        ccp = pltpu.make_async_copy(c_hbm, cv, csem.at[0])
        if nodma & 1:
            class _N:
                def start(self): pass
                def wait(self): pass
            ccp = _N()
            wcp = lambda c: _N()
            xcps = [[_N()]] * len(xpieces)
        for c in WSCH[0]:
            wcp(c).start()
        ccp.start()
        xs[pl.ds(0, HEAD), :] = jnp.zeros((HEAD, D), bf16)
        for b in range(B):
            xs[pl.ds(b * BSTR + HEAD + T, BSTR - T), :] = jnp.zeros((BSTR - T, D), bf16)
        for sl in range(WSL):
            for k in range(K, 32):
                wv[sl, k] = jnp.zeros((16, D2), bf16)

        def start_x(js):
            for j in js:
                for c in xcps[j]:
                    c.start()

        def wait_x(js):
            for j in js:
                for c in xcps[j]:
                    c.wait()

        ccp.wait()

        def wunit(jg):
            sl = jg % WSL
            for e in range(ET):
                wd = pltpu.bitcast(wv[sl, :, :, e * 128:(e + 1) * 128], u32)
                wd = jnp.swapaxes(wd, 0, 1)
                rhs = jnp.concatenate([pltpu.bitcast(wd[2 * t:2 * t + 2].reshape(64, 128), bf16) for t in range(4)], 1)
                rc = RC + (e // DT) * 4 * N
                res = jnp.dot(cv[rc:rc + 4 * N, :], rhs, preferred_element_type=f32)
                for jj in range(2):
                    for fo in range(8):
                        r0 = (jj * 8 + fo) * 32
                        for t in range(4):
                            m = []
                            for dd in range(2):
                                vr = res[r0 + dd * 16:r0 + dd * 16 + 8, t * 128:(t + 1) * 128]
                                vi = res[r0 + dd * 16 + 8:r0 + dd * 16 + 16, t * 128:(t + 1) * 128]
                                m.append((vr, vi - vr, vi + vr))
                            for cc in range(3):
                                W3[e, pl.ds((cc * NF + fo * 8) * HP + jg * 8 + 2 * t + jj, 8, stride=HP), :] = _pack(m[0][cc], m[1][cc])

        def wbody(it, carry):
            for t in range(uw):
                wcp(it * uw + t).wait()
            for i in range(NWI):
                if i + 1 < len(WSCH) or XSCH[i]:
                    @pl.when(it == i)
                    def _():
                        if i + 1 < len(WSCH):
                            for c in WSCH[i + 1]:
                                wcp(c).start()
                        start_x(XSCH[i])
            for t in range(uw):
                wunit(it * uw + t)
            return carry
        lax.fori_loop(0, NWI, wbody, 0)

        def s1(il):
            r0 = pl.multiple_of(il * HOP, HOP)
            cols = []
            for d in range(DT):
                xw = pltpu.bitcast(xs[pl.ds(r0, 2 * N), d * 128:(d + 1) * 128], u32)
                cols.append([v.astype(bf16) for v in _unpack(xw)])
            rhs = jnp.concatenate([cols[d][p] for d in range(DT) for p in range(2)], 1)
            res = jnp.dot(cv[RF:RF + N, :], rhs, preferred_element_type=f32)
            for d in range(DT):
                ev = res[:, (2 * d) * 128:(2 * d + 1) * 128]
                od = res[:, (2 * d + 1) * 128:(2 * d + 2) * 128]
                m = [(v[:NF] + v[NF:], v[:NF], v[NF:]) for v in (ev, od)]
                for c in range(3):
                    Xh[d, pl.ds(c * NF * P + il, NF, stride=P), :] = _pack(m[0][c], m[1][c])
            return res

        def xcopy(s, il, g=None):
            r0 = pl.multiple_of((s * NB + il) * HOP + HEAD, 64)
            xw = pltpu.bitcast(xs[pl.ds(r0, HOP), :], u32)
            if g is not None:
                xw = jnp.where(g[0], pltpu.bitcast(g[1][0][:, :D], u32), xw)
            for d in range(DT):
                xu[d, pl.ds(il * XP + HIST + 4, L), :] = xw[:, d * 128:(d + 1) * 128]

        def xhead(s):
            xw = pltpu.bitcast(xs[pl.ds(pl.multiple_of(s * NB * HOP, 64), HEAD), :], u32)
            for d in range(DT):
                xu[d, pl.ds(0, HIST), :] = xw[:, d * 128:(d + 1) * 128]

        XR = 3 * NF * P // NCS
        assert XR * NCS == 3 * NF * P and XR % 8 == 0

        def xmove(i, t, g=None):
            per = (XR // 8 // u3) * 8
            r0 = t * per
            n = per if t < u3 - 1 else XR - r0
            r = pl.multiple_of(i * XR + r0, 8)
            for d in range(DT):
                v = Xn[d, pl.ds(r, n), :]
                if g is not None:
                    gv = pltpu.bitcast(g[1][1][:, (2 + d) * 128:(3 + d) * 128], u32)
                    v = jnp.concatenate([jnp.where(g[0], gv[(q * 8) % L:(q * 8) % L + 8], v[q * 8:q * 8 + 8]) for q in range(n // 8)], 0)
                Xh[d, pl.ds(r, n), :] = v

        gates = []

        def fftunit(unit, never):
            rg = unit // DT
            d = unit % DT
            base = rg * (8 * XP)

            def gate():
                return gates.pop(0) if gates else None

            def words(n, p, g):
                wd = xu[d, pl.ds(base + n + (4 if n >= HIST else 0), 8, stride=XP), :]
                if g is None:
                    return pltpu.unpack_elementwise(wd, index=p, packed_dtype=bf16, unpacked_dtype=f32)
                if p == 0:
                    return pltpu.bitcast(wd << jnp.where(never, g, jnp.uint32(16)), f32)
                return pltpu.bitcast(wd & jnp.where(never, g, jnp.uint32(0xFFFF0000)), f32)

            def tst(i, v):
                TT[pl.ds(i * 8, 8), :] = v

            def tld(i, g):
                v = TT[pl.ds(i * 8, 8), :]
                return v if g is None else jnp.where(never, pltpu.bitcast(g, f32), v)

            def emit(g, v):
                m = [(a + b_, a, b_) for (a, b_) in v]
                for c in range(3):
                    Xn[d, pl.ds((c * NF + g) * P + rg * 8, 8), :] = _pack(m[0][c], m[1][c])
            return _fwd128(words, tst, tld, emit, gate)

        def s2(f, tick):
            k = []
            for c in range(3):
                r = (c * NF + f) * P
                lhs = jnp.concatenate([pltpu.bitcast(Xh[d, pl.ds(r, NB), :], bf16) for d in range(DT)], 1)
                rw = (c * NF + f) * HP
                wf = jnp.concatenate([pltpu.bitcast(W3[e, pl.ds(rw, H), :], bf16) for e in range(ET)], 1)
                k.append(jnp.dot(lhs, wf, preferred_element_type=f32))
                tick(k[-1])
            p = _pack(k[0] - k[2], k[0] + k[1])
            for e in range(ET):
                Yh[e, pl.ds(f * PY, 2 * NB), :] = p[:, e * 128:(e + 1) * 128]

        def s3(il):
            z = []
            for p in range(2):
                yw = jnp.concatenate([pltpu.bitcast(Yh[e, pl.ds(2 * il + p, NF, stride=PY), :], bf16) for e in range(ET)], 1)
                z.append(jnp.dot(cv[RG:RG + L, :], yw, preferred_element_type=f32))
            outs = []
            for p in range(2):
                tf = jnp.tanh(z[p][:, :D]) * 0.5
                outs.append(tf + tf * jnp.tanh(z[p][:, D:]))
            ost[pl.ds(pl.multiple_of(il * HOP, HOP), HOP), :] = pltpu.bitcast(_pack(outs[0], outs[1]), bf16)
            return z

        def out_copy(s, i):
            ch = s * NCS + i
            b = ch // CPB
            t0 = pl.multiple_of((ch % CPB) * CH, CH)
            n = pl.multiple_of(jnp.where((ch % CPB) == CPB - 1, CHL, CH), 64)
            return pltpu.make_async_copy(ost.at[pl.ds(pl.multiple_of(i * CH, CH), n)],
                                         o_hbm.at[b, pl.ds(t0, n)], osem.at[i])

        start_x(xlate)
        wait_x(range(PPS))
        h1 = NB // 2

        def body1(il, carry):
            s1(il)
            return carry
        lax.fori_loop(0, h1, body1, 0, unroll=u1)
        wait_x(range(PPS, 2 * PPS))
        start_x(range(2 * PPS, NQ // XB))
        xhead(1)

        def body1x(i, carry):
            res = s1(h1 + i)
            nv = z_ref[0] > 0
            xcopy(1, 2 * i, (nv, [res[:L, :D]]) if XG else None)
            xcopy(1, 2 * i + 1, (nv, [res[:L, D:]]) if XG else None)
            return carry
        lax.fori_loop(0, NB - h1, body1x, 0, unroll=u1)

        def sbody(s, carry):
            never = z_ref[0] > 0

            def s2b(i, carry):
                def chain():
                    for u in range(FU):
                        yield from fftunit(i * FU + u, never)
                gen = chain()
                npieces = FU * 32
                st = [0, 0]

                def tick(kk):
                    st[0] += 1
                    n_ = (st[0] * npieces) // (3 * u2) - st[1]
                    del gates[:]
                    for z_ in range(n_):
                        ph = (z_ + GOFF) / n_ * len(GT)
                        tl = GT[int(ph)]
                        rr = int((ph % 1.0) * (NB // 4))
                        gates.append(pltpu.bitcast(kk[rr * 8:rr * 8 + 8, tl * 128:(tl + 1) * 128], u32))
                    for _ in range(n_):
                        next(gen, None)
                        st[1] += 1
                for t in range(u2):
                    s2(i * u2 + t, tick)
                for _ in gen:
                    pass
                return carry
            lax.fori_loop(0, NI2, s2b, 0)

            sx = jnp.minimum(s + 2, NS - 1)
            for ss in range(2, NS):
                @pl.when(s == ss - 2)
                def _():
                    wait_x(range(ss * PPS, (ss + 1) * PPS))
            xhead(sx)

            if not nodma & 2:
                @pl.when(s > 0)
                def _():
                    def owait(i, carry):
                        out_copy(s - 1, i).wait()
                        return carry
                    lax.fori_loop(0, NCS, owait, 0)

            mcp = pltpu.make_async_copy(Xn, Xh, msem.at[0])
            if XMV == 'dma':
                mcp.start()

            def body3(i, carry):
                for t in range(u3):
                    il = i * u3 + t
                    zz = s3(il)
                    xcopy(sx, il, (never, zz) if XG else None)
                    if XMV != 'dma':
                        xmove(i, t, (never, zz) if XG > 1 else None)
                if not nodma & 2:
                    out_copy(s, i).start()
                return carry
            lax.fori_loop(0, jnp.where(s < NS - 1, NCS, nl // u3), body3, 0)
            if XMV == 'dma':
                mcp.wait()
            return carry
        lax.fori_loop(0, NS, sbody, 0)

        lcps = []
        il = nl
        for n in LCS:
            for t in range(n):
                s3(il + t)
            if not nodma & 2:
                q0 = (NS - 1) * NB + il
                b, i0 = divmod(q0, nblk)
                t0 = i0 * HOP
                nr = min(n * HOP, T - t0)
                cp = pltpu.make_async_copy(ost.at[pl.ds(il * HOP, nr)], o_hbm.at[b, pl.ds(t0, nr)], lsem.at[len(lcps)])
                cp.start()
                lcps.append(cp)
            il += n
        if not nodma & 2:
            for i in range(nl // u3):
                out_copy(jnp.int32(NS - 1), jnp.int32(i)).wait()
            for cp in lcps:
                cp.wait()

    def fn(x, w):
        return pl.pallas_call(
            kernel,
            in_specs=[pl.BlockSpec(memory_space=pl.ANY)] * 3 + [pl.BlockSpec(memory_space=pltpu.SMEM)],
            out_specs=pl.BlockSpec(memory_space=pl.ANY),
            out_shape=jax.ShapeDtypeStruct((B, T, D), x.dtype),
            scratch_shapes=[
                pltpu.VMEM((XROWS, D), bf16),
                pltpu.VMEM((WSL, 32, 16, D2), bf16),
                pltpu.VMEM((ET, 3 * NF * HP, 128), u32),
                pltpu.VMEM((DT, 3 * NF * P, 128), u32),
                pltpu.VMEM((DT, 3 * NF * P, 128), u32),
                pltpu.VMEM((ET, NF * PY, 128), u32),
                pltpu.VMEM((NB * HOP, D), bf16),
                pltpu.VMEM(consts.shape, bf16),
                pltpu.VMEM((DT, NB * XP + HIST + 8, 128), u32),
                pltpu.VMEM((2048, 128), f32),
                pltpu.SemaphoreType.DMA((WSL,)),
                pltpu.SemaphoreType.DMA((nxs,)),
                pltpu.SemaphoreType.DMA((NCS,)),
                pltpu.SemaphoreType.DMA((len(LCS),)),
                pltpu.SemaphoreType.DMA((1,)),
                pltpu.SemaphoreType.DMA((1,)),
            ],
            compiler_params=pltpu.CompilerParams(vmem_limit_bytes=127 * 1024 * 1024, flags=flags),
        )(x, w, consts, np.zeros((1,), np.int32))
    return fn


@jax.jit
def pallas_standalone__autoregressive_conv_wavernn__speech_kernel(x, w):
    B, T, D = x.shape
    K = w.shape[0]
    return make(B, T, D, K, )(x, w)
```

```python
import math
import numpy as np
import jax
import jax.numpy as jnp
from jax import lax
import jax.experimental.pallas as pl
import jax.experimental.pallas.tpu as pltpu

N = 128
L = 96
HIST = N - L
NF = N // 2
bf16 = jnp.bfloat16
u32 = jnp.uint32
f32 = jnp.float32


def _consts(K):
    th = np.pi * (4 * np.arange(NF) + 1) / N
    n = np.arange(N)
    F = np.concatenate([np.cos(th[:, None] * n), np.sin(th[:, None] * n)], 0)
    m = np.arange(L) + HIST
    G = np.zeros((L, NF, 2)); G[:, :, 0] = np.cos(th[None] * m[:, None]) * 2 / N
    G[:, :, 1] = np.sin(th[None] * m[:, None]) * 2 / N
    G = G.reshape(L, N)
    j = (K - 1) - np.arange(K)
    C = np.zeros((N, 32))
    C[:NF, :K] = np.cos(th[:, None] * j); C[NF:, :K] = np.sin(th[:, None] * j)
    Cb = np.zeros((2, 4 * N, 128))
    for jj in range(2):
        for dd in range(2):
            g = 2 * jj + dd
            Cb[0, g * N:(g + 1) * N, jj * 64 + dd:(jj + 1) * 64:2] = C
    Cb = Cb.reshape(2, 2, 2, 2, 8, 8, 128).transpose(0, 1, 4, 2, 3, 5, 6).reshape(2, 4 * N, 128)
    Cb[1] = 0.5 * Cb[0]
    return np.asarray(np.concatenate([F, Cb[0], Cb[1], G], 0), dtype=bf16)


def _unpack(x):
    return [pltpu.unpack_elementwise(x, index=i, packed_dtype=bf16, unpacked_dtype=f32) for i in range(2)]


def _pack(a, b):
    return pltpu.pack_elementwise([a, b], packed_dtype=bf16)


def _cmul(re, im, w):
    c, s = w.real, w.imag
    eps = 1e-12
    def close(a, b): return abs(a - b) < eps
    if close(c, 1) and close(s, 0): return re, im
    if close(c, -1) and close(s, 0): return -re, -im
    if close(c, 0) and close(s, 1): return -im, re
    if close(c, 0) and close(s, -1): return im, -re
    if close(abs(c), abs(s)):
        a = c
        if close(s, c):
            return (re - im) * a, (re + im) * a
        else:
            return (re + im) * a, (im - re) * a
    return re * c - im * s, re * s + im * c

def _fft(xs, sign=-1):
    n = len(xs)
    if n == 1: return xs
    if n == 2:
        (a, b), (c, d) = xs
        return [(a + c, b + d), (a - c, b - d)]
    if n == 4:
        (a0, b0), (a1, b1), (a2, b2), (a3, b3) = xs
        s0r, s0i, d0r, d0i = a0 + a2, b0 + b2, a0 - a2, b0 - b2
        s1r, s1i, d1r, d1i = a1 + a3, b1 + b3, a1 - a3, b1 - b3
        if sign < 0:
            return [(s0r + s1r, s0i + s1i), (d0r + d1i, d0i - d1r), (s0r - s1r, s0i - s1i), (d0r - d1i, d0i + d1r)]
        return [(s0r + s1r, s0i + s1i), (d0r - d1i, d0i + d1r), (s0r - s1r, s0i - s1i), (d0r + d1i, d0i - d1r)]
    ev = _fft(xs[0::2], sign); od = _fft(xs[1::2], sign)
    out = [None] * n
    for k in range(n // 2):
        w = complex(math.cos(2 * math.pi * k / n), sign * math.sin(2 * math.pi * k / n))
        if abs(w.real) < 1e-12 and abs(w.imag - sign) < 1e-12:
            r, i_ = od[k]
            if sign < 0:
                out[k] = (ev[k][0] + i_, ev[k][1] - r); out[k + n // 2] = (ev[k][0] - i_, ev[k][1] + r)
            else:
                out[k] = (ev[k][0] - i_, ev[k][1] + r); out[k + n // 2] = (ev[k][0] + i_, ev[k][1] - r)
            continue
        tr, ti = _cmul(od[k][0], od[k][1], w)
        out[k] = (ev[k][0] + tr, ev[k][1] + ti)
        out[k + n // 2] = (ev[k][0] - tr, ev[k][1] - ti)
    return out

def _rot(ph):
    return complex(math.cos(ph), math.sin(ph))


def _fwd128(loadw, tst, tld, emit, gate):
    for n2 in range(8):
        for p in range(2):
            g = gate()
            col = []
            for n1 in range(8):
                a = loadw(8 * n1 + n2, p, g); b = loadw(8 * n1 + n2 + 64, p, g)
                col.append(_cmul(a, b, _rot(math.pi * 8 * n1 / 128)))
            o = _fft(col, +1)
            for g1 in range(8):
                r, i_ = _cmul(o[g1][0], o[g1][1], _rot(2 * math.pi * g1 * n2 / 64 + math.pi * n2 / 128))
                tst(((p * 8 + g1) * 8 + n2) * 2, r); tst(((p * 8 + g1) * 8 + n2) * 2 + 1, i_)
            yield
    for g1 in range(8):
        for p in range(2):
            g = gate()
            o = _fft([(tld(((p * 8 + g1) * 8 + n2) * 2, g), tld(((p * 8 + g1) * 8 + n2) * 2 + 1, g)) for n2 in range(8)], +1)
            if p == 0:
                o0 = o
            else:
                for g2 in range(8):
                    emit(g1 + 8 * g2, [o0[g2], o[g2]])
            yield


def make(B, T, D, K, NB=56, u1=28, u2=32, u3=28, uw=2, nodma=0, LCS=(4,) * 7, XAT=4, WSL=8,
         GT=(0, 2), GOFF=0.0, flags=None, XMV='v', XG=2, XSCH=None, WSCH=None, SUB=(4,) * 7):
    HOP = 2 * L
    nblk = -(-T // HOP)
    NQ = B * nblk
    assert NQ % NB == 0 and NB % 8 == 0
    NS = NQ // NB
    BSTR = nblk * HOP
    HEAD = 2 * HIST
    XROWS = NQ * HOP + HEAD
    D2 = 2 * D
    ET = D2 // 128
    DT = D // 128
    H = D // 2
    HP = H + 1
    P = NB + 1 if NB % 8 == 0 else NB
    PY = 2 * NB + 1
    XP = L + 4
    OCB = u3
    assert nblk % OCB == 0 and NB % u3 == 0
    CPB = nblk // OCB
    CH = OCB * HOP
    CHL = T - (CPB - 1) * CH
    assert sum(SUB) == OCB and CHL > sum(SUB[:-1]) * HOP
    SUBE = [sum(SUB[:j + 1]) for j in range(len(SUB))]
    NCS = NB // OCB
    WC = D // 16
    NWI = WC // uw
    if WSCH is None:
        WSCH = [[0, 1], [2, 3, 4], [5, 6, 7], [8, 9], [10, 11], [12, 13], [14, 15]]
    for i, z in enumerate(WSCH[1:]):
        assert all(c < i * uw + WSL for c in z)
    nl = NB - sum(LCS)
    assert nl % u3 == 0 and sum(LCS) == u3
    NU = (NB // 8) * DT
    NI2 = NF // u2
    assert NU % NI2 == 0
    FU = NU // NI2

    XB = 8
    xpieces = []
    for j in range(NQ // XB):
        lo, hi = j * XB * HOP + HEAD, (j + 1) * XB * HOP + HEAD
        parts = []
        for b in range(B):
            r0, r1 = max(lo, b * BSTR + HEAD), min(hi, b * BSTR + HEAD + T)
            if r1 > r0:
                parts.append((b, r0 - b * BSTR - HEAD, r1 - r0))
        xpieces.append(parts)
    PPS = NB // XB
    if XSCH is None:
        XSCH = [[], [0, 1], [2, 3], [4, 5], [6, 7], [8, 9], [10, 11], [12, 13]]
    xlate = [j for j in range(2 * PPS) if not any(j in z for z in XSCH)]
    nxs = sum(len(p) for p in xpieces)

    consts = _consts(K)
    RF, RC, RG = 0, N, N + 8 * N

    def kernel(x_hbm, w_hbm, c_hbm, z_ref, o_hbm, xs, wv, W3, Xh, Xn, Yh, ost, cv, xu, TT, wsem, xsem, osem, lsem, csem, msem):
        def wcp(c):
            r = c * 16 if isinstance(c, int) else pl.multiple_of(c * 16, 16)
            return pltpu.make_async_copy(w_hbm.at[:, pl.ds(r, 16), :], wv.at[c % WSL, pl.ds(0, K)], wsem.at[c % WSL])

        xcps = []
        for parts in xpieces:
            xcps.append([pltpu.make_async_copy(x_hbm.at[b, pl.ds(t0, n), :], xs.at[pl.ds(b * BSTR + HEAD + t0, n), :],
                                               xsem.at[sum(map(len, xcps)) + i]) for i, (b, t0, n) in enumerate(parts)])
        ccp = pltpu.make_async_copy(c_hbm, cv, csem.at[0])
        if nodma & 1:
            class _N:
                def start(self): pass
                def wait(self): pass
            ccp = _N()
            wcp = lambda c: _N()
            xcps = [[_N()]] * len(xpieces)
        for c in WSCH[0]:
            wcp(c).start()
        ccp.start()
        xs[pl.ds(0, HEAD), :] = jnp.zeros((HEAD, D), bf16)
        for b in range(B):
            xs[pl.ds(b * BSTR + HEAD + T, BSTR - T), :] = jnp.zeros((BSTR - T, D), bf16)
        for sl in range(WSL):
            for k in range(K, 32):
                wv[sl, k] = jnp.zeros((16, D2), bf16)

        def start_x(js):
            for j in js:
                for c in xcps[j]:
                    c.start()

        def wait_x(js):
            for j in js:
                for c in xcps[j]:
                    c.wait()

        ccp.wait()

        def wunit(jg):
            sl = jg % WSL
            for e in range(ET):
                wd = pltpu.bitcast(wv[sl, :, :, e * 128:(e + 1) * 128], u32)
                wd = jnp.swapaxes(wd, 0, 1)
                rhs = jnp.concatenate([pltpu.bitcast(wd[2 * t:2 * t + 2].reshape(64, 128), bf16) for t in range(4)], 1)
                rc = RC + (e // DT) * 4 * N
                res = jnp.dot(cv[rc:rc + 4 * N, :], rhs, preferred_element_type=f32)
                for jj in range(2):
                    for fo in range(8):
                        r0 = (jj * 8 + fo) * 32
                        for t in range(4):
                            m = []
                            for dd in range(2):
                                vr = res[r0 + dd * 16:r0 + dd * 16 + 8, t * 128:(t + 1) * 128]
                                vi = res[r0 + dd * 16 + 8:r0 + dd * 16 + 16, t * 128:(t + 1) * 128]
                                m.append((vr, vi - vr, vi + vr))
                            for cc in range(3):
                                W3[e, pl.ds((cc * NF + fo * 8) * HP + jg * 8 + 2 * t + jj, 8, stride=HP), :] = _pack(m[0][cc], m[1][cc])

        def wbody(it, carry):
            for t in range(uw):
                wcp(it * uw + t).wait()
            for i in range(NWI):
                if i + 1 < len(WSCH) or XSCH[i]:
                    @pl.when(it == i)
                    def _():
                        if i + 1 < len(WSCH):
                            for c in WSCH[i + 1]:
                                wcp(c).start()
                        start_x(XSCH[i])
            for t in range(uw):
                wunit(it * uw + t)
            return carry
        lax.fori_loop(0, NWI, wbody, 0)

        def s1(il):
            r0 = pl.multiple_of(il * HOP, HOP)
            cols = []
            for d in range(DT):
                xw = pltpu.bitcast(xs[pl.ds(r0, 2 * N), d * 128:(d + 1) * 128], u32)
                cols.append([v.astype(bf16) for v in _unpack(xw)])
            rhs = jnp.concatenate([cols[d][p] for d in range(DT) for p in range(2)], 1)
            res = jnp.dot(cv[RF:RF + N, :], rhs, preferred_element_type=f32)
            for d in range(DT):
                ev = res[:, (2 * d) * 128:(2 * d + 1) * 128]
                od = res[:, (2 * d + 1) * 128:(2 * d + 2) * 128]
                m = [(v[:NF] + v[NF:], v[:NF], v[NF:]) for v in (ev, od)]
                for c in range(3):
                    Xh[d, pl.ds(c * NF * P + il, NF, stride=P), :] = _pack(m[0][c], m[1][c])
            return res

        def xcopy(s, il, g=None):
            r0 = pl.multiple_of((s * NB + il) * HOP + HEAD, 64)
            xw = pltpu.bitcast(xs[pl.ds(r0, HOP), :], u32)
            if g is not None:
                xw = jnp.where(g[0], pltpu.bitcast(g[1][0][:, :D], u32), xw)
            for d in range(DT):
                xu[d, pl.ds(il * XP + HIST + 4, L), :] = xw[:, d * 128:(d + 1) * 128]

        def xhead(s):
            xw = pltpu.bitcast(xs[pl.ds(pl.multiple_of(s * NB * HOP, 64), HEAD), :], u32)
            for d in range(DT):
                xu[d, pl.ds(0, HIST), :] = xw[:, d * 128:(d + 1) * 128]

        XR = 3 * NF * P // NCS
        assert XR * NCS == 3 * NF * P and XR % 8 == 0

        def xmove(i, t, g=None):
            per = (XR // 8 // u3) * 8
            r0 = t * per
            n = per if t < u3 - 1 else XR - r0
            r = pl.multiple_of(i * XR + r0, 8)
            for d in range(DT):
                v = Xn[d, pl.ds(r, n), :]
                if g is not None:
                    gv = pltpu.bitcast(g[1][1][:, (2 + d) * 128:(3 + d) * 128], u32)
                    v = jnp.concatenate([jnp.where(g[0], gv[(q * 8) % L:(q * 8) % L + 8], v[q * 8:q * 8 + 8]) for q in range(n // 8)], 0)
                Xh[d, pl.ds(r, n), :] = v

        gates = []

        def fftunit(unit, never):
            rg = unit // DT
            d = unit % DT
            base = rg * (8 * XP)

            def gate():
                return gates.pop(0) if gates else None

            def words(n, p, g):
                wd = xu[d, pl.ds(base + n + (4 if n >= HIST else 0), 8, stride=XP), :]
                if g is None:
                    return pltpu.unpack_elementwise(wd, index=p, packed_dtype=bf16, unpacked_dtype=f32)
                if p == 0:
                    return pltpu.bitcast(wd << jnp.where(never, g, jnp.uint32(16)), f32)
                return pltpu.bitcast(wd & jnp.where(never, g, jnp.uint32(0xFFFF0000)), f32)

            def tst(i, v):
                TT[pl.ds(i * 8, 8), :] = v

            def tld(i, g):
                v = TT[pl.ds(i * 8, 8), :]
                return v if g is None else jnp.where(never, pltpu.bitcast(g, f32), v)

            def emit(g, v):
                m = [(a + b_, a, b_) for (a, b_) in v]
                for c in range(3):
                    Xn[d, pl.ds((c * NF + g) * P + rg * 8, 8), :] = _pack(m[0][c], m[1][c])
            return _fwd128(words, tst, tld, emit, gate)

        def s2(f, tick):
            k = []
            for c in range(3):
                r = (c * NF + f) * P
                lhs = jnp.concatenate([pltpu.bitcast(Xh[d, pl.ds(r, NB), :], bf16) for d in range(DT)], 1)
                rw = (c * NF + f) * HP
                wf = jnp.concatenate([pltpu.bitcast(W3[e, pl.ds(rw, H), :], bf16) for e in range(ET)], 1)
                k.append(jnp.dot(lhs, wf, preferred_element_type=f32))
                tick(k[-1])
            p = _pack(k[0] - k[2], k[0] + k[1])
            for e in range(ET):
                Yh[e, pl.ds(f * PY, 2 * NB), :] = p[:, e * 128:(e + 1) * 128]

        def s3(il):
            z = []
            for p in range(2):
                yw = jnp.concatenate([pltpu.bitcast(Yh[e, pl.ds(2 * il + p, NF, stride=PY), :], bf16) for e in range(ET)], 1)
                z.append(jnp.dot(cv[RG:RG + L, :], yw, preferred_element_type=f32))
            outs = []
            for p in range(2):
                tf = jnp.tanh(z[p][:, :D]) * 0.5
                outs.append(tf + tf * jnp.tanh(z[p][:, D:]))
            ost[pl.ds(pl.multiple_of(il * HOP, HOP), HOP), :] = pltpu.bitcast(_pack(outs[0], outs[1]), bf16)
            return z

        def out_copy(s, i, j):
            ch = s * NCS + i
            b = ch // CPB
            o = sum(SUB[:j]) * HOP
            t0 = pl.multiple_of((ch % CPB) * CH + o, 64)
            n = SUB[j] * HOP
            if j == len(SUB) - 1:
                n = pl.multiple_of(jnp.where((ch % CPB) == CPB - 1, CHL - o, n), 64)
            return pltpu.make_async_copy(ost.at[pl.ds(pl.multiple_of(i * CH + o, 64), n)],
                                         o_hbm.at[b, pl.ds(t0, n)], osem.at[i * len(SUB) + j])

        start_x(xlate)
        wait_x(range(PPS))
        h1 = NB // 2

        def body1(il, carry):
            s1(il)
            return carry
        lax.fori_loop(0, h1, body1, 0, unroll=u1)
        wait_x(range(PPS, 2 * PPS))
        start_x(range(2 * PPS, NQ // XB))
        xhead(1)

        def body1x(i, carry):
            res = s1(h1 + i)
            nv = z_ref[0] > 0
            xcopy(1, 2 * i, (nv, [res[:L, :D]]) if XG else None)
            xcopy(1, 2 * i + 1, (nv, [res[:L, D:]]) if XG else None)
            return carry
        lax.fori_loop(0, NB - h1, body1x, 0, unroll=u1)

        def sbody(s, carry):
            never = z_ref[0] > 0

            def s2b(i, carry):
                def chain():
                    for u in range(FU):
                        yield from fftunit(i * FU + u, never)
                gen = chain()
                npieces = FU * 32
                st = [0, 0]

                def tick(kk):
                    st[0] += 1
                    n_ = (st[0] * npieces) // (3 * u2) - st[1]
                    del gates[:]
                    for z_ in range(n_):
                        ph = (z_ + GOFF) / n_ * len(GT)
                        tl = GT[int(ph)]
                        rr = int((ph % 1.0) * (NB // 4))
                        gates.append(pltpu.bitcast(kk[rr * 8:rr * 8 + 8, tl * 128:(tl + 1) * 128], u32))
                    for _ in range(n_):
                        next(gen, None)
                        st[1] += 1
                for t in range(u2):
                    s2(i * u2 + t, tick)
                for _ in gen:
                    pass
                return carry
            lax.fori_loop(0, NI2, s2b, 0)

            sx = jnp.minimum(s + 2, NS - 1)
            for ss in range(2, NS):
                @pl.when(s == ss - 2)
                def _():
                    wait_x(range(ss * PPS, (ss + 1) * PPS))
            xhead(sx)

            if not nodma & 2:
                @pl.when(s > 0)
                def _():
                    def owait(i, carry):
                        for j in range(len(SUB)):
                            out_copy(s - 1, i, j).wait()
                        return carry
                    lax.fori_loop(0, NCS, owait, 0)

            mcp = pltpu.make_async_copy(Xn, Xh, msem.at[0])
            if XMV == 'dma':
                mcp.start()

            def body3(i, carry):
                for t in range(u3):
                    il = i * u3 + t
                    zz = s3(il)
                    xcopy(sx, il, (never, zz) if XG else None)
                    if XMV != 'dma':
                        xmove(i, t, (never, zz) if XG > 1 else None)
                    if not nodma & 2 and (t + 1) in SUBE:
                        out_copy(s, i, SUBE.index(t + 1)).start()
                return carry
            lax.fori_loop(0, jnp.where(s < NS - 1, NCS, nl // u3), body3, 0)
            if XMV == 'dma':
                mcp.wait()
            return carry
        lax.fori_loop(0, NS, sbody, 0)

        lcps = []
        il = nl
        for n in LCS:
            for t in range(n):
                s3(il + t)
            if not nodma & 2:
                q0 = (NS - 1) * NB + il
                b, i0 = divmod(q0, nblk)
                t0 = i0 * HOP
                nr = min(n * HOP, T - t0)
                cp = pltpu.make_async_copy(ost.at[pl.ds(il * HOP, nr)], o_hbm.at[b, pl.ds(t0, nr)], lsem.at[len(lcps)])
                cp.start()
                lcps.append(cp)
            il += n
        if not nodma & 2:
            for i in range(nl // u3):
                for j in range(len(SUB)):
                    out_copy(jnp.int32(NS - 1), jnp.int32(i), j).wait()
            for cp in lcps:
                cp.wait()

    def fn(x, w):
        return pl.pallas_call(
            kernel,
            in_specs=[pl.BlockSpec(memory_space=pl.ANY)] * 3 + [pl.BlockSpec(memory_space=pltpu.SMEM)],
            out_specs=pl.BlockSpec(memory_space=pl.ANY),
            out_shape=jax.ShapeDtypeStruct((B, T, D), x.dtype),
            scratch_shapes=[
                pltpu.VMEM((XROWS, D), bf16),
                pltpu.VMEM((WSL, 32, 16, D2), bf16),
                pltpu.VMEM((ET, 3 * NF * HP, 128), u32),
                pltpu.VMEM((DT, 3 * NF * P, 128), u32),
                pltpu.VMEM((DT, 3 * NF * P, 128), u32),
                pltpu.VMEM((ET, NF * PY, 128), u32),
                pltpu.VMEM((NB * HOP, D), bf16),
                pltpu.VMEM(consts.shape, bf16),
                pltpu.VMEM((DT, NB * XP + HIST + 8, 128), u32),
                pltpu.VMEM((2048, 128), f32),
                pltpu.SemaphoreType.DMA((WSL,)),
                pltpu.SemaphoreType.DMA((nxs,)),
                pltpu.SemaphoreType.DMA((NCS * len(SUB),)),
                pltpu.SemaphoreType.DMA((len(LCS),)),
                pltpu.SemaphoreType.DMA((1,)),
                pltpu.SemaphoreType.DMA((1,)),
            ],
            compiler_params=pltpu.CompilerParams(vmem_limit_bytes=127 * 1024 * 1024, flags=flags),
        )(x, w, consts, np.zeros((1,), np.int32))
    return fn


@jax.jit
def pallas_standalone__autoregressive_conv_wavernn__speech_kernel(x, w):
    B, T, D = x.shape
    K = w.shape[0]
    return make(B, T, D, K, )(x, w)
```

```python
import math
import numpy as np
import jax
import jax.numpy as jnp
from jax import lax
import jax.experimental.pallas as pl
import jax.experimental.pallas.tpu as pltpu

N = 128
L = 96
HIST = N - L
NF = N // 2
bf16 = jnp.bfloat16
u32 = jnp.uint32
f32 = jnp.float32


def _consts(K):
    th = np.pi * (4 * np.arange(NF) + 1) / N
    n = np.arange(N)
    F = np.concatenate([np.cos(th[:, None] * n), np.sin(th[:, None] * n)], 0)
    m = np.arange(L) + HIST
    G = np.zeros((L, NF, 2)); G[:, :, 0] = np.cos(th[None] * m[:, None]) * 2 / N
    G[:, :, 1] = np.sin(th[None] * m[:, None]) * 2 / N
    G = G.reshape(L, N)
    j = (K - 1) - np.arange(K)
    C = np.zeros((N, 32))
    C[:NF, :K] = np.cos(th[:, None] * j); C[NF:, :K] = np.sin(th[:, None] * j)
    Cb = np.zeros((2, 4 * N, 128))
    for jj in range(2):
        for dd in range(2):
            g = 2 * jj + dd
            Cb[0, g * N:(g + 1) * N, jj * 64 + dd:(jj + 1) * 64:2] = C
    Cb = Cb.reshape(2, 2, 2, 2, 8, 8, 128).transpose(0, 1, 4, 2, 3, 5, 6).reshape(2, 4 * N, 128)
    Cb[1] = 0.5 * Cb[0]
    return np.asarray(np.concatenate([F, Cb[0], Cb[1], G], 0), dtype=bf16)


def _unpack(x):
    return [pltpu.unpack_elementwise(x, index=i, packed_dtype=bf16, unpacked_dtype=f32) for i in range(2)]


def _pack(a, b):
    return pltpu.pack_elementwise([a, b], packed_dtype=bf16)


def _cmul(re, im, w):
    c, s = w.real, w.imag
    eps = 1e-12
    def close(a, b): return abs(a - b) < eps
    if close(c, 1) and close(s, 0): return re, im
    if close(c, -1) and close(s, 0): return -re, -im
    if close(c, 0) and close(s, 1): return -im, re
    if close(c, 0) and close(s, -1): return im, -re
    if close(abs(c), abs(s)):
        a = c
        if close(s, c):
            return (re - im) * a, (re + im) * a
        else:
            return (re + im) * a, (im - re) * a
    return re * c - im * s, re * s + im * c

def _fft(xs, sign=-1):
    n = len(xs)
    if n == 1: return xs
    if n == 2:
        (a, b), (c, d) = xs
        return [(a + c, b + d), (a - c, b - d)]
    if n == 4:
        (a0, b0), (a1, b1), (a2, b2), (a3, b3) = xs
        s0r, s0i, d0r, d0i = a0 + a2, b0 + b2, a0 - a2, b0 - b2
        s1r, s1i, d1r, d1i = a1 + a3, b1 + b3, a1 - a3, b1 - b3
        if sign < 0:
            return [(s0r + s1r, s0i + s1i), (d0r + d1i, d0i - d1r), (s0r - s1r, s0i - s1i), (d0r - d1i, d0i + d1r)]
        return [(s0r + s1r, s0i + s1i), (d0r - d1i, d0i + d1r), (s0r - s1r, s0i - s1i), (d0r + d1i, d0i - d1r)]
    ev = _fft(xs[0::2], sign); od = _fft(xs[1::2], sign)
    out = [None] * n
    for k in range(n // 2):
        w = complex(math.cos(2 * math.pi * k / n), sign * math.sin(2 * math.pi * k / n))
        if abs(w.real) < 1e-12 and abs(w.imag - sign) < 1e-12:
            r, i_ = od[k]
            if sign < 0:
                out[k] = (ev[k][0] + i_, ev[k][1] - r); out[k + n // 2] = (ev[k][0] - i_, ev[k][1] + r)
            else:
                out[k] = (ev[k][0] - i_, ev[k][1] + r); out[k + n // 2] = (ev[k][0] + i_, ev[k][1] - r)
            continue
        tr, ti = _cmul(od[k][0], od[k][1], w)
        out[k] = (ev[k][0] + tr, ev[k][1] + ti)
        out[k + n // 2] = (ev[k][0] - tr, ev[k][1] - ti)
    return out

def _rot(ph):
    return complex(math.cos(ph), math.sin(ph))


def _fwd128(loadw, tst, tld, emit, gate):
    for n2 in range(8):
        for p in range(2):
            g = gate()
            col = []
            for n1 in range(8):
                a = loadw(8 * n1 + n2, p, g); b = loadw(8 * n1 + n2 + 64, p, g)
                col.append(_cmul(a, b, _rot(math.pi * 8 * n1 / 128)))
            o = _fft(col, +1)
            for g1 in range(8):
                r, i_ = _cmul(o[g1][0], o[g1][1], _rot(2 * math.pi * g1 * n2 / 64 + math.pi * n2 / 128))
                tst(((p * 8 + g1) * 8 + n2) * 2, r); tst(((p * 8 + g1) * 8 + n2) * 2 + 1, i_)
            yield
    for g1 in range(8):
        for p in range(2):
            g = gate()
            o = _fft([(tld(((p * 8 + g1) * 8 + n2) * 2, g), tld(((p * 8 + g1) * 8 + n2) * 2 + 1, g)) for n2 in range(8)], +1)
            if p == 0:
                o0 = o
            else:
                for g2 in range(8):
                    emit(g1 + 8 * g2, [o0[g2], o[g2]])
            yield


def _inv128(loadw, tst, tld, emit, gate, sc):
    for gb in range(8):
        g = gate()
        o = _fft([loadw(8 * ga + gb, g) for ga in range(8)], -1)
        for k1 in range(8):
            r, i_ = _cmul(o[k1][0], o[k1][1], sc * _rot(-2 * math.pi * gb * k1 / 64 - math.pi * k1 / 128))
            tst((k1 * 8 + gb) * 2, r); tst((k1 * 8 + gb) * 2 + 1, i_)
        yield
    for k1 in range(8):
        g = gate()
        o = _fft([(tld((k1 * 8 + gb) * 2, g), tld((k1 * 8 + gb) * 2 + 1, g)) for gb in range(8)], -1)
        for k2 in range(8):
            n = k1 + 8 * k2
            w = _rot(-math.pi * k2 / 16)
            re, im = o[k2]
            if n >= 32:
                r, i_ = _cmul(re, im, w)
                emit(n, r, g)
            else:
                i_ = im if k2 == 0 else re * w.imag + im * w.real
            emit(n + 64, i_, g)
        yield


def make(B, T, D, K, NB=56, u1=28, u2=32, u3=28, uw=2, nodma=0, XAT=4, WSL=8,
         GT=(0, 2), GOFF=0.0, flags=None, XMV='v', XG=2, XSCH=None, WSCH=None, RGV=4, IFR=0.9, OG=4):
    HOP = 2 * L
    nblk = -(-T // HOP)
    NQ = B * nblk
    assert NQ % NB == 0 and NB % 8 == 0
    NS = NQ // NB
    BSTR = nblk * HOP
    HEAD = 2 * HIST
    XROWS = NQ * HOP + HEAD
    D2 = 2 * D
    ET = D2 // 128
    DT = D // 128
    H = D // 2
    HP = H + 1
    P = NB + 1 if NB % 8 == 0 else NB
    PY = 2 * NB + 1
    XP = L + 4
    assert nblk % OG == 0 and NB % u3 == 0 and u3 % OG == 0 and 8 % OG == 0
    NG = NB // OG
    NCS = NB // u3
    NV = 8 * RGV
    PB = 2 * NV + 1
    assert NS >= 2 and (ET // DT) * NF * PB <= 3 * NF * P
    WC = D // 16
    NWI = WC // uw
    if WSCH is None:
        WSCH = [[0, 1], [2, 3, 4], [5, 6, 7], [8, 9], [10, 11], [12, 13], [14, 15]]
    for i, z in enumerate(WSCH[1:]):
        assert all(c < i * uw + WSL for c in z)
    NU = (NB // 8) * DT
    NI2 = NF // u2
    assert NU % NI2 == 0
    FU = NU // NI2
    assert (RGV * DT) % NI2 == 0
    assert (RGV * DT // NI2) % DT == 0
    IU = RGV * DT // NI2

    XB = 8
    xpieces = []
    for j in range(NQ // XB):
        lo, hi = j * XB * HOP + HEAD, (j + 1) * XB * HOP + HEAD
        parts = []
        for b in range(B):
            r0, r1 = max(lo, b * BSTR + HEAD), min(hi, b * BSTR + HEAD + T)
            if r1 > r0:
                parts.append((b, r0 - b * BSTR - HEAD, r1 - r0))
        xpieces.append(parts)
    PPS = NB // XB
    if XSCH is None:
        XSCH = [[], [0, 1], [2, 3], [4, 5], [6, 7], [8, 9], [10, 11], [12, 13]]
    xlate = [j for j in range(2 * PPS) if not any(j in z for z in XSCH)]
    nxs = sum(len(p) for p in xpieces)

    consts = _consts(K)
    RF, RC, RG = 0, N, N + 8 * N

    def kernel(x_hbm, w_hbm, c_hbm, z_ref, o_hbm, xs, wv, W3, Xh, Xn, Yh, ost, ost2, cv, xu, TT, SG, SO, ou, wsem, xsem, osem, o2sem, csem):
        def wcp(c):
            r = c * 16 if isinstance(c, int) else pl.multiple_of(c * 16, 16)
            return pltpu.make_async_copy(w_hbm.at[:, pl.ds(r, 16), :], wv.at[c % WSL, pl.ds(0, K)], wsem.at[c % WSL])

        xcps = []
        for parts in xpieces:
            xcps.append([pltpu.make_async_copy(x_hbm.at[b, pl.ds(t0, n), :], xs.at[pl.ds(b * BSTR + HEAD + t0, n), :],
                                               xsem.at[sum(map(len, xcps)) + i]) for i, (b, t0, n) in enumerate(parts)])
        ccp = pltpu.make_async_copy(c_hbm, cv, csem.at[0])
        if nodma & 1:
            class _N:
                def start(self): pass
                def wait(self): pass
            ccp = _N()
            wcp = lambda c: _N()
            xcps = [[_N()]] * len(xpieces)
        for c in WSCH[0]:
            wcp(c).start()
        ccp.start()
        xs[pl.ds(0, HEAD), :] = jnp.zeros((HEAD, D), bf16)
        for b in range(B):
            xs[pl.ds(b * BSTR + HEAD + T, BSTR - T), :] = jnp.zeros((BSTR - T, D), bf16)
        for sl in range(WSL):
            for k in range(K, 32):
                wv[sl, k] = jnp.zeros((16, D2), bf16)

        def start_x(js):
            for j in js:
                for c in xcps[j]:
                    c.start()

        def wait_x(js):
            for j in js:
                for c in xcps[j]:
                    c.wait()

        ccp.wait()

        def wunit(jg):
            sl = jg % WSL
            for e in range(ET):
                wd = pltpu.bitcast(wv[sl, :, :, e * 128:(e + 1) * 128], u32)
                wd = jnp.swapaxes(wd, 0, 1)
                rhs = jnp.concatenate([pltpu.bitcast(wd[2 * t:2 * t + 2].reshape(64, 128), bf16) for t in range(4)], 1)
                rc = RC + (e // DT) * 4 * N
                res = jnp.dot(cv[rc:rc + 4 * N, :], rhs, preferred_element_type=f32)
                for jj in range(2):
                    for fo in range(8):
                        r0 = (jj * 8 + fo) * 32
                        for t in range(4):
                            m = []
                            for dd in range(2):
                                vr = res[r0 + dd * 16:r0 + dd * 16 + 8, t * 128:(t + 1) * 128]
                                vi = res[r0 + dd * 16 + 8:r0 + dd * 16 + 16, t * 128:(t + 1) * 128]
                                m.append((vr, vi - vr, vi + vr))
                            for cc in range(3):
                                W3[e, pl.ds((cc * NF + fo * 8) * HP + jg * 8 + 2 * t + jj, 8, stride=HP), :] = _pack(m[0][cc], m[1][cc])

        def wbody(it, carry):
            for t in range(uw):
                wcp(it * uw + t).wait()
            for i in range(NWI):
                if i + 1 < len(WSCH) or XSCH[i]:
                    @pl.when(it == i)
                    def _():
                        if i + 1 < len(WSCH):
                            for c in WSCH[i + 1]:
                                wcp(c).start()
                        start_x(XSCH[i])
            for t in range(uw):
                wunit(it * uw + t)
            return carry
        lax.fori_loop(0, NWI, wbody, 0)

        def s1(il):
            r0 = pl.multiple_of(il * HOP, HOP)
            cols = []
            for d in range(DT):
                xw = pltpu.bitcast(xs[pl.ds(r0, 2 * N), d * 128:(d + 1) * 128], u32)
                cols.append([v.astype(bf16) for v in _unpack(xw)])
            rhs = jnp.concatenate([cols[d][p] for d in range(DT) for p in range(2)], 1)
            res = jnp.dot(cv[RF:RF + N, :], rhs, preferred_element_type=f32)
            for d in range(DT):
                ev = res[:, (2 * d) * 128:(2 * d + 1) * 128]
                od = res[:, (2 * d + 1) * 128:(2 * d + 2) * 128]
                m = [(v[:NF] + v[NF:], v[:NF], v[NF:]) for v in (ev, od)]
                for c in range(3):
                    Xh[d, pl.ds(c * NF * P + il, NF, stride=P), :] = _pack(m[0][c], m[1][c])
            return res

        def xcopy(s, il, g=None):
            r0 = pl.multiple_of((s * NB + il) * HOP + HEAD, 64)
            xw = pltpu.bitcast(xs[pl.ds(r0, HOP), :], u32)
            if g is not None:
                xw = jnp.where(g[0], pltpu.bitcast(g[1][0][:, :D], u32), xw)
            for d in range(DT):
                xu[d, pl.ds(il * XP + HIST + 4, L), :] = xw[:, d * 128:(d + 1) * 128]

        def xhead(s):
            xw = pltpu.bitcast(xs[pl.ds(pl.multiple_of(s * NB * HOP, 64), HEAD), :], u32)
            for d in range(DT):
                xu[d, pl.ds(0, HIST), :] = xw[:, d * 128:(d + 1) * 128]

        XR = 3 * NF * P // NCS
        assert XR * NCS == 3 * NF * P and XR % 8 == 0

        def xmove(i, t, g=None):
            per = (XR // 8 // u3) * 8
            r0 = t * per
            n = per if t < u3 - 1 else XR - r0
            r = pl.multiple_of(i * XR + r0, 8)
            for d in range(DT):
                v = Xn[d, pl.ds(r, n), :]
                if g is not None:
                    gv = pltpu.bitcast(g[1][1][:, (2 + d) * 128:(3 + d) * 128], u32)
                    v = jnp.concatenate([jnp.where(g[0], gv[(q * 8) % L:(q * 8) % L + 8], v[q * 8:q * 8 + 8]) for q in range(n // 8)], 0)
                Xh[d, pl.ds(r, n), :] = v

        gates = []

        def fftunit(unit, never):
            rg = unit // DT
            d = unit % DT
            base = rg * (8 * XP)

            def gate():
                return gates.pop(0) if gates else None

            def words(n, p, g):
                wd = xu[d, pl.ds(base + n + (4 if n >= HIST else 0), 8, stride=XP), :]
                if g is None:
                    return pltpu.unpack_elementwise(wd, index=p, packed_dtype=bf16, unpacked_dtype=f32)
                if p == 0:
                    return pltpu.bitcast(wd << jnp.where(never, g, jnp.uint32(16)), f32)
                return pltpu.bitcast(wd & jnp.where(never, g, jnp.uint32(0xFFFF0000)), f32)

            def tst(i, v):
                TT[pl.ds(i * 8, 8), :] = v

            def tld(i, g):
                v = TT[pl.ds(i * 8, 8), :]
                return v if g is None else jnp.where(never, pltpu.bitcast(g, f32), v)

            def emit(g, v):
                m = [(a + b_, a, b_) for (a, b_) in v]
                for c in range(3):
                    Xn[d, pl.ds((c * NF + g) * P + rg * 8, 8), :] = _pack(m[0][c], m[1][c])
            return _fwd128(words, tst, tld, emit, gate)

        def s2(Xs, f, tick):
            k = []
            for c in range(3):
                r = (c * NF + f) * P
                lhs = jnp.concatenate([pltpu.bitcast(Xs[d, pl.ds(r, NB), :], bf16) for d in range(DT)], 1)
                rw = (c * NF + f) * HP
                wf = jnp.concatenate([pltpu.bitcast(W3[e, pl.ds(rw, H), :], bf16) for e in range(ET)], 1)
                k.append(jnp.dot(lhs, wf, preferred_element_type=f32))
                tick(k[-1])
            p = _pack(k[0] - k[2], k[0] + k[1])
            for e in range(ET):
                Yh[e, pl.ds(f * PY, 2 * NB), :] = p[:, e * 128:(e + 1) * 128]

        def s3(il):
            z = []
            for p in range(2):
                yw = jnp.concatenate([pltpu.bitcast(Yh[e, pl.ds(2 * il + p, NF, stride=PY), :], bf16) for e in range(ET)], 1)
                z.append(jnp.dot(cv[RG:RG + L, :], yw, preferred_element_type=f32))
            outs = []
            for p in range(2):
                tf = jnp.tanh(z[p][:, :D]) * 0.5
                outs.append(tf + tf * jnp.tanh(z[p][:, D:]))
            ost[pl.ds(pl.multiple_of(il * HOP, HOP), HOP), :] = pltpu.bitcast(_pack(outs[0], outs[1]), bf16)
            return z

        def ocp(src, row, q, sem):
            b = q // nblk
            t0 = pl.multiple_of((q % nblk) * HOP, 64)
            n = pl.multiple_of(jnp.minimum(OG * HOP, T - t0), 64)
            return pltpu.make_async_copy(src.at[pl.ds(pl.multiple_of(row, 64), n)], o_hbm.at[b, pl.ds(t0, n)], sem)

        def out_copy(s, gi):
            s = jnp.int32(s) if isinstance(s, int) else s
            gi = jnp.int32(gi) if isinstance(gi, int) else gi
            return ocp(ost, gi * (OG * HOP), s * NB + gi * OG, osem.at[gi])

        def out2_copy(gi):
            gi = jnp.int32(gi) if isinstance(gi, int) else gi
            return ocp(ost2, gi * (OG * HOP), (NS - 2) * NB + gi * OG, o2sem.at[gi])

        start_x(xlate)
        wait_x(range(PPS))
        h1 = NB // 2

        def body1(il, carry):
            s1(il)
            return carry
        lax.fori_loop(0, h1, body1, 0, unroll=u1)
        wait_x(range(PPS, 2 * PPS))
        start_x(range(2 * PPS, NQ // XB))
        xhead(1)

        def body1x(i, carry):
            res = s1(h1 + i)
            nv = z_ref[0] > 0
            xcopy(1, 2 * i, (nv, [res[:L, :D]]) if XG else None)
            xcopy(1, 2 * i + 1, (nv, [res[:L, D:]]) if XG else None)
            return carry
        lax.fori_loop(0, NB - h1, body1x, 0, unroll=u1)

        def run_s2(Xsrc, units, npu, frac):
            def s2b(i, carry):
                us = units(i)

                def chain():
                    for u in us:
                        yield from u
                gen = chain()
                npieces = len(us) * npu
                st = [0, 0]
                nt = int(3 * u2 * frac)

                def tick(kk):
                    st[0] += 1
                    n_ = min(npieces, (st[0] * npieces) // nt) - st[1]
                    del gates[:]
                    for z_ in range(n_):
                        ph = (z_ + GOFF) / n_ * len(GT)
                        tl = GT[int(ph)]
                        rr = int((ph % 1.0) * (NB // 4))
                        gates.append(pltpu.bitcast(kk[rr * 8:rr * 8 + 8, tl * 128:(tl + 1) * 128], u32))
                    for _ in range(n_):
                        next(gen, None)
                        st[1] += 1
                for t in range(u2):
                    s2(Xsrc, i * u2 + t, tick)
                assert st[1] == npieces
                for _ in gen:
                    pass
                return carry
            lax.fori_loop(0, NI2, s2b, 0)

        def gsel(never, g, v):
            n = v.shape[0] // 8
            return jnp.concatenate([jnp.where(never, g[(q * 8) % L:(q * 8) % L + 8], v[q * 8:q * 8 + 8]) for q in range(n)], 0)

        def ifftunit(unit, a, never):
            rg = unit // DT

            def gate():
                return gates.pop(0) if gates else None

            def sel(g, v):
                return v if g is None else jnp.where(never, pltpu.bitcast(g, v.dtype), v)

            def tst(i, v):
                TT[pl.ds(i * 8, 8), :] = v

            def tld(i, g):
                return sel(g, TT[pl.ds(i * 8, 8), :])

            for p in range(2):
                for half in (1, 0):
                    def loadw(gi, g):
                        wd = Xh[half, pl.ds((a * NF + gi) * PB + rg * 16 + p, 8, stride=2), :]
                        if g is None:
                            return tuple(_unpack(wd))
                        return (pltpu.bitcast(wd << jnp.where(never, g, jnp.uint32(16)), f32),
                                pltpu.bitcast(wd & jnp.where(never, g, jnp.uint32(0xFFFF0000)), f32))

                    def emit(m, z, g):
                        r = (m - HIST) * 8
                        if half == 1:
                            SG[pl.ds(r, 8), :] = jnp.tanh(z)
                        else:
                            tf = jnp.tanh(z) * 0.5
                            o = tf + tf * sel(g, SG[pl.ds(r, 8), :])
                            if p == 0:
                                SO[pl.ds(r, 8), :] = o
                            else:
                                ou[pl.ds(m - HIST, 8, stride=XP), :] = _pack(sel(g, SO[pl.ds(r, 8), :]), o)
                    yield from _inv128(loadw, tst, tld, emit, gate, 2.0 / N)
            for b2 in range(4):
                g = gate()
                for b8 in (2 * b2, 2 * b2 + 1):
                    wd = ou[pl.ds(b8 * XP, L), :]
                    if g is not None:
                        wd = jnp.concatenate([jnp.where(never, g, wd[q * 8:q * 8 + 8]) for q in range(L // 8)], 0)
                    ost2[pl.ds(pl.multiple_of((rg * 8 + b8) * HOP, HOP), HOP), a * 128:(a + 1) * 128] = pltpu.bitcast(wd, bf16)
                yield
            if a == DT - 1 and not nodma & 2:
                for j in range(8 // OG):
                    out2_copy(rg * (8 // OG) + j).start()

        def sbody(s, carry):
            never = z_ref[0] > 0

            @pl.when(s < NS - 1)
            def _():
                run_s2(Xh, lambda i: [fftunit(i * FU + u, never) for u in range(FU)], 32, 1.0)

            @pl.when(s == NS - 1)
            def _():
                run_s2(Xn, lambda i: [ifftunit(i * IU + u, u % DT, never) for u in range(IU)], 68, IFR)

            for ss in range(2, NS):
                @pl.when(s == ss - 2)
                def _():
                    wait_x(range(ss * PPS, (ss + 1) * PPS))

            if not nodma & 2:
                @pl.when(s > 0)
                def _():
                    def owait(gi, carry):
                        out_copy(s - 1, gi).wait()
                        return carry
                    lax.fori_loop(jnp.where(s == NS - 1, NV // OG, 0), NG, owait, 0)

            @pl.when(s != NS - 2)
            def _():
                sx = jnp.minimum(s + 2, NS - 1)
                xhead(sx)

                def body3(i, carry):
                    for t in range(u3):
                        il = i * u3 + t
                        zz = s3(il)
                        xcopy(sx, il, (never, zz))
                        xmove(i, t, (never, zz))
                        if not nodma & 2 and (t + 1) % OG == 0:
                            out_copy(s, i * (u3 // OG) + t // OG).start()
                    return carry
                lax.fori_loop(0, NCS, body3, 0)

            @pl.when(s == NS - 2)
            def _():
                nm = NB - NV
                ncp = ET * NF
                for t in range(nm):
                    il = NV + t
                    zz = s3(il)
                    for q in range(t * ncp // nm, (t + 1) * ncp // nm):
                        e, g = divmod(q, NF)
                        gv = pltpu.bitcast(zz[q % 2][:, e * 128:(e + 1) * 128], u32)
                        Xh[e // DT, pl.ds(((e % DT) * NF + g) * PB, 2 * NV), :] = gsel(never, gv, Yh[e, pl.ds(g * PY, 2 * NV), :])
                    if not nodma & 2 and (il + 1) % OG == 0:
                        out_copy(s, il // OG).start()
            return carry
        lax.fori_loop(0, NS, sbody, 0)

        if not nodma & 2:
            for gi in range(NV // OG):
                out2_copy(gi).wait()
            for gi in range(NG):
                out_copy(NS - 1, gi).wait()

    def fn(x, w):
        return pl.pallas_call(
            kernel,
            in_specs=[pl.BlockSpec(memory_space=pl.ANY)] * 3 + [pl.BlockSpec(memory_space=pltpu.SMEM)],
            out_specs=pl.BlockSpec(memory_space=pl.ANY),
            out_shape=jax.ShapeDtypeStruct((B, T, D), x.dtype),
            scratch_shapes=[
                pltpu.VMEM((XROWS, D), bf16),
                pltpu.VMEM((WSL, 32, 16, D2), bf16),
                pltpu.VMEM((ET, 3 * NF * HP, 128), u32),
                pltpu.VMEM((DT, 3 * NF * P, 128), u32),
                pltpu.VMEM((DT, 3 * NF * P, 128), u32),
                pltpu.VMEM((ET, NF * PY, 128), u32),
                pltpu.VMEM((NB * HOP, D), bf16),
                pltpu.VMEM((NV * HOP, D), bf16),
                pltpu.VMEM(consts.shape, bf16),
                pltpu.VMEM((DT, NB * XP + HIST + 8, 128), u32),
                pltpu.VMEM((2048, 128), f32),
                pltpu.VMEM((L * 8, 128), f32),
                pltpu.VMEM((L * 8, 128), f32),
                pltpu.VMEM((8 * XP, 128), u32),
                pltpu.SemaphoreType.DMA((WSL,)),
                pltpu.SemaphoreType.DMA((nxs,)),
                pltpu.SemaphoreType.DMA((NG,)),
                pltpu.SemaphoreType.DMA((NV // OG,)),
                pltpu.SemaphoreType.DMA((1,)),
            ],
            compiler_params=pltpu.CompilerParams(vmem_limit_bytes=127 * 1024 * 1024, flags=flags),
        )(x, w, consts, np.zeros((1,), np.int32))
    return fn


@jax.jit
def pallas_standalone__autoregressive_conv_wavernn__speech_kernel(x, w):
    B, T, D = x.shape
    K = w.shape[0]
    return make(B, T, D, K, )(x, w)
```

```python
import math
import numpy as np
import jax
import jax.numpy as jnp
from jax import lax
import jax.experimental.pallas as pl
import jax.experimental.pallas.tpu as pltpu

N = 128
L = 96
HIST = N - L
NF = N // 2
bf16 = jnp.bfloat16
u32 = jnp.uint32
f32 = jnp.float32


def _consts(K):
    th = np.pi * (4 * np.arange(NF) + 1) / N
    n = np.arange(N)
    F = np.concatenate([np.cos(th[:, None] * n), np.sin(th[:, None] * n)], 0)
    m = np.arange(L) + HIST
    G = np.zeros((L, NF, 2)); G[:, :, 0] = np.cos(th[None] * m[:, None]) * 2 / N
    G[:, :, 1] = np.sin(th[None] * m[:, None]) * 2 / N
    G = G.reshape(L, N)
    j = (K - 1) - np.arange(K)
    C = np.zeros((N, 32))
    C[:NF, :K] = np.cos(th[:, None] * j); C[NF:, :K] = np.sin(th[:, None] * j)
    Cb = np.zeros((2, 4 * N, 128))
    for jj in range(2):
        for dd in range(2):
            g = 2 * jj + dd
            Cb[0, g * N:(g + 1) * N, jj * 64 + dd:(jj + 1) * 64:2] = C
    Cb = Cb.reshape(2, 2, 2, 2, 8, 8, 128).transpose(0, 1, 4, 2, 3, 5, 6).reshape(2, 4 * N, 128)
    Cb[1] = 0.5 * Cb[0]
    return np.asarray(np.concatenate([F, Cb[0], Cb[1], G], 0), dtype=bf16)


def _unpack(x):
    return [pltpu.unpack_elementwise(x, index=i, packed_dtype=bf16, unpacked_dtype=f32) for i in range(2)]


def _pack(a, b):
    return pltpu.pack_elementwise([a, b], packed_dtype=bf16)


def _cmul(re, im, w):
    c, s = w.real, w.imag
    eps = 1e-12
    def close(a, b): return abs(a - b) < eps
    if close(c, 1) and close(s, 0): return re, im
    if close(c, -1) and close(s, 0): return -re, -im
    if close(c, 0) and close(s, 1): return -im, re
    if close(c, 0) and close(s, -1): return im, -re
    if close(abs(c), abs(s)):
        a = c
        if close(s, c):
            return (re - im) * a, (re + im) * a
        else:
            return (re + im) * a, (im - re) * a
    return re * c - im * s, re * s + im * c

def _fft(xs, sign=-1):
    n = len(xs)
    if n == 1: return xs
    if n == 2:
        (a, b), (c, d) = xs
        return [(a + c, b + d), (a - c, b - d)]
    if n == 4:
        (a0, b0), (a1, b1), (a2, b2), (a3, b3) = xs
        s0r, s0i, d0r, d0i = a0 + a2, b0 + b2, a0 - a2, b0 - b2
        s1r, s1i, d1r, d1i = a1 + a3, b1 + b3, a1 - a3, b1 - b3
        if sign < 0:
            return [(s0r + s1r, s0i + s1i), (d0r + d1i, d0i - d1r), (s0r - s1r, s0i - s1i), (d0r - d1i, d0i + d1r)]
        return [(s0r + s1r, s0i + s1i), (d0r - d1i, d0i + d1r), (s0r - s1r, s0i - s1i), (d0r + d1i, d0i - d1r)]
    ev = _fft(xs[0::2], sign); od = _fft(xs[1::2], sign)
    out = [None] * n
    for k in range(n // 2):
        w = complex(math.cos(2 * math.pi * k / n), sign * math.sin(2 * math.pi * k / n))
        if abs(w.real) < 1e-12 and abs(w.imag - sign) < 1e-12:
            r, i_ = od[k]
            if sign < 0:
                out[k] = (ev[k][0] + i_, ev[k][1] - r); out[k + n // 2] = (ev[k][0] - i_, ev[k][1] + r)
            else:
                out[k] = (ev[k][0] - i_, ev[k][1] + r); out[k + n // 2] = (ev[k][0] + i_, ev[k][1] - r)
            continue
        tr, ti = _cmul(od[k][0], od[k][1], w)
        out[k] = (ev[k][0] + tr, ev[k][1] + ti)
        out[k + n // 2] = (ev[k][0] - tr, ev[k][1] - ti)
    return out

def _rot(ph):
    return complex(math.cos(ph), math.sin(ph))


def _fwd128(loadw, tst, tld, emit, gate, HG=1):
    for n2 in range(8):
        for p in range(2):
            g = gate()
            col = []
            for n1 in range(8):
                a = loadw(8 * n1 + n2, p, g); b = loadw(8 * n1 + n2 + 64, p, g)
                col.append(_cmul(a, b, _rot(math.pi * 8 * n1 / 128)))
            o = _fft(col, +1)
            for g1 in range(8):
                r, i_ = _cmul(o[g1][0], o[g1][1], _rot(2 * math.pi * g1 * n2 / 64 + math.pi * n2 / 128))
                tst(((p * 8 + g1) * 8 + n2) * 2, r); tst(((p * 8 + g1) * 8 + n2) * 2 + 1, i_)
            yield
    for g1 in range(8):
        for p in range(2):
            g = gate()
            o = _fft([(tld(((p * 8 + g1) * 8 + n2) * 2, g if (n2 < 4 or not HG) else None), tld(((p * 8 + g1) * 8 + n2) * 2 + 1, g if (n2 < 4 or not HG) else None)) for n2 in range(8)], +1)
            if p == 0:
                o0 = o
            else:
                for g2 in range(8):
                    emit(g1 + 8 * g2, [o0[g2], o[g2]])
            yield


def _inv128(loadw, tst, tld, emit, gate, sc, HG=1):
    for gb in range(8):
        g = gate()
        o = _fft([loadw(8 * ga + gb, g) for ga in range(8)], -1)
        for k1 in range(8):
            r, i_ = _cmul(o[k1][0], o[k1][1], sc * _rot(-2 * math.pi * gb * k1 / 64 - math.pi * k1 / 128))
            tst((k1 * 8 + gb) * 2, r); tst((k1 * 8 + gb) * 2 + 1, i_)
        yield
    for k1 in range(8):
        g = gate()
        o = _fft([(tld((k1 * 8 + gb) * 2, g if (gb < 4 or not HG) else None), tld((k1 * 8 + gb) * 2 + 1, g if (gb < 4 or not HG) else None)) for gb in range(8)], -1)
        for k2 in range(8):
            n = k1 + 8 * k2
            w = _rot(-math.pi * k2 / 16)
            re, im = o[k2]
            if n >= 32:
                r, i_ = _cmul(re, im, w)
                emit(n, r, g)
            else:
                i_ = im if k2 == 0 else re * w.imag + im * w.real
            emit(n + 64, i_, g)
        yield


def make(B, T, D, K, NB=56, u1=28, u2=32, u3=28, uw=2, WSL=8,
         GT=(0, 2), GOFF=0.25, XSCH=None, WSCH=None, RGV=4, IFR=0.94, OG=4, CPL=1, HG=0, FFR=0.94):
    HOP = 2 * L
    nblk = -(-T // HOP)
    NQ = B * nblk
    assert NQ % NB == 0 and NB % 8 == 0
    NS = NQ // NB
    BSTR = nblk * HOP
    HEAD = 2 * HIST
    XROWS = NQ * HOP + HEAD
    D2 = 2 * D
    ET = D2 // 128
    DT = D // 128
    H = D // 2
    HP = H + 1
    P = NB + 1 if NB % 8 == 0 else NB
    PY = 2 * NB + 1
    XP = L + 4
    assert nblk % OG == 0 and NB % u3 == 0 and u3 % OG == 0 and 8 % OG == 0
    NG = NB // OG
    NCS = NB // u3
    NV = 8 * RGV
    PB = 2 * NV + 1
    assert NS >= 2 and (ET // DT) * NF * PB <= 3 * NF * P
    WC = D // 16
    NWI = WC // uw
    if WSCH is None:
        WSCH = [[0, 1], [2, 3, 4], [5, 6, 7], [8, 9], [10, 11], [12, 13], [14, 15]]
    for i, z in enumerate(WSCH[1:]):
        assert all(c < i * uw + WSL for c in z)
    NU = (NB // 8) * DT
    NI2 = NF // u2
    assert NU % NI2 == 0
    FU = NU // NI2
    assert (RGV * DT) % NI2 == 0
    assert (RGV * DT // NI2) % DT == 0
    IU = RGV * DT // NI2

    XB = 8
    xpieces = []
    for j in range(NQ // XB):
        lo, hi = j * XB * HOP + HEAD, (j + 1) * XB * HOP + HEAD
        parts = []
        for b in range(B):
            r0, r1 = max(lo, b * BSTR + HEAD), min(hi, b * BSTR + HEAD + T)
            if r1 > r0:
                parts.append((b, r0 - b * BSTR - HEAD, r1 - r0))
        xpieces.append(parts)
    PPS = NB // XB
    if XSCH is None:
        XSCH = [[], [0, 1], [2, 3], [4, 5], [6, 7], [8, 9], [10, 11], [12, 13]]
    xlate = [j for j in range(2 * PPS) if not any(j in z for z in XSCH)]
    nxs = sum(len(p) for p in xpieces)

    consts = _consts(K)
    RF, RC, RG = 0, N, N + 8 * N

    def kernel(x_hbm, w_hbm, c_hbm, z_ref, o_hbm, xs, wv, W3, Xh, Xn, Yh, ost, ost2, cv, xu, TT, SG, SO, ou, wsem, xsem, osem, o2sem, csem):
        def wcp(c):
            r = c * 16 if isinstance(c, int) else pl.multiple_of(c * 16, 16)
            return pltpu.make_async_copy(w_hbm.at[:, pl.ds(r, 16), :], wv.at[c % WSL, pl.ds(0, K)], wsem.at[c % WSL])

        xcps = []
        for parts in xpieces:
            xcps.append([pltpu.make_async_copy(x_hbm.at[b, pl.ds(t0, n), :], xs.at[pl.ds(b * BSTR + HEAD + t0, n), :],
                                               xsem.at[sum(map(len, xcps)) + i]) for i, (b, t0, n) in enumerate(parts)])
        ccp = pltpu.make_async_copy(c_hbm, cv, csem.at[0])
        for c in WSCH[0]:
            wcp(c).start()
        ccp.start()
        xs[pl.ds(0, HEAD), :] = jnp.zeros((HEAD, D), bf16)
        for b in range(B):
            xs[pl.ds(b * BSTR + HEAD + T, BSTR - T), :] = jnp.zeros((BSTR - T, D), bf16)
        for sl in range(WSL):
            for k in range(K, 32):
                wv[sl, k] = jnp.zeros((16, D2), bf16)

        def start_x(js):
            for j in js:
                for c in xcps[j]:
                    c.start()

        def wait_x(js):
            for j in js:
                for c in xcps[j]:
                    c.wait()

        ccp.wait()

        def wunit(jg):
            sl = jg % WSL
            for e in range(ET):
                wd = pltpu.bitcast(wv[sl, :, :, e * 128:(e + 1) * 128], u32)
                wd = jnp.swapaxes(wd, 0, 1)
                rhs = jnp.concatenate([pltpu.bitcast(wd[2 * t:2 * t + 2].reshape(64, 128), bf16) for t in range(4)], 1)
                rc = RC + (e // DT) * 4 * N
                res = jnp.dot(cv[rc:rc + 4 * N, :], rhs, preferred_element_type=f32)
                for jj in range(2):
                    for fo in range(8):
                        r0 = (jj * 8 + fo) * 32
                        for t in range(4):
                            m = []
                            for dd in range(2):
                                vr = res[r0 + dd * 16:r0 + dd * 16 + 8, t * 128:(t + 1) * 128]
                                vi = res[r0 + dd * 16 + 8:r0 + dd * 16 + 16, t * 128:(t + 1) * 128]
                                m.append((vr, vi - vr, vi + vr))
                            for cc in range(3):
                                W3[e, pl.ds((cc * NF + fo * 8) * HP + jg * 8 + 2 * t + jj, 8, stride=HP), :] = _pack(m[0][cc], m[1][cc])

        def wbody(it, carry):
            for t in range(uw):
                wcp(it * uw + t).wait()
            for i in range(NWI):
                if i + 1 < len(WSCH) or XSCH[i]:
                    @pl.when(it == i)
                    def _():
                        if i + 1 < len(WSCH):
                            for c in WSCH[i + 1]:
                                wcp(c).start()
                        start_x(XSCH[i])
            for t in range(uw):
                wunit(it * uw + t)
            return carry
        lax.fori_loop(0, NWI, wbody, 0)

        def s1(il):
            r0 = pl.multiple_of(il * HOP, HOP)
            cols = []
            for d in range(DT):
                xw = pltpu.bitcast(xs[pl.ds(r0, 2 * N), d * 128:(d + 1) * 128], u32)
                cols.append([v.astype(bf16) for v in _unpack(xw)])
            rhs = jnp.concatenate([cols[d][p] for d in range(DT) for p in range(2)], 1)
            res = jnp.dot(cv[RF:RF + N, :], rhs, preferred_element_type=f32)
            for d in range(DT):
                ev = res[:, (2 * d) * 128:(2 * d + 1) * 128]
                od = res[:, (2 * d + 1) * 128:(2 * d + 2) * 128]
                m = [(v[:NF] + v[NF:], v[:NF], v[NF:]) for v in (ev, od)]
                for c in range(3):
                    Xh[d, pl.ds(c * NF * P + il, NF, stride=P), :] = _pack(m[0][c], m[1][c])
            return res

        def xcopy(s, il, g=None):
            r0 = pl.multiple_of((s * NB + il) * HOP + HEAD, 64)
            xw = pltpu.bitcast(xs[pl.ds(r0, HOP), :], u32)
            if g is not None:
                xw = jnp.where(g[0], pltpu.bitcast(g[1][0][:, :D], u32), xw)
            for d in range(DT):
                xu[d, pl.ds(il * XP + HIST + 4, L), :] = xw[:, d * 128:(d + 1) * 128]

        def xhead(s):
            xw = pltpu.bitcast(xs[pl.ds(pl.multiple_of(s * NB * HOP, 64), HEAD), :], u32)
            for d in range(DT):
                xu[d, pl.ds(0, HIST), :] = xw[:, d * 128:(d + 1) * 128]

        XR = 3 * NF * P // NCS
        assert XR * NCS == 3 * NF * P and XR % 8 == 0

        def xmove(i, t, g=None):
            per = (XR // 8 // u3) * 8
            r0 = t * per
            n = per if t < u3 - 1 else XR - r0
            r = pl.multiple_of(i * XR + r0, 8)
            for d in range(DT):
                v = Xn[d, pl.ds(r, n), :]
                if g is not None:
                    gv = pltpu.bitcast(g[1][1][:, (2 + d) * 128:(3 + d) * 128], u32)
                    v = jnp.concatenate([jnp.where(g[0], gv[(q * 8) % L:(q * 8) % L + 8], v[q * 8:q * 8 + 8]) for q in range(n // 8)], 0)
                Xh[d, pl.ds(r, n), :] = v

        gates = []

        def fftunit(unit, never):
            rg = unit // DT
            d = unit % DT
            base = rg * (8 * XP)

            def gate():
                return gates.pop(0) if gates else None

            def words(n, p, g):
                wd = xu[d, pl.ds(base + n + (4 if n >= HIST else 0), 8, stride=XP), :]
                if g is None:
                    return pltpu.unpack_elementwise(wd, index=p, packed_dtype=bf16, unpacked_dtype=f32)
                if p == 0:
                    return pltpu.bitcast(wd << jnp.where(never, g, jnp.uint32(16)), f32)
                return pltpu.bitcast(wd & jnp.where(never, g, jnp.uint32(0xFFFF0000)), f32)

            def tst(i, v):
                TT[pl.ds(i * 8, 8), :] = v

            def tld(i, g):
                v = TT[pl.ds(i * 8, 8), :]
                return v if g is None else jnp.where(never, pltpu.bitcast(g, f32), v)

            def emit(g, v):
                m = [(a + b_, a, b_) for (a, b_) in v]
                for c in range(3):
                    Xn[d, pl.ds((c * NF + g) * P + rg * 8, 8), :] = _pack(m[0][c], m[1][c])
            return _fwd128(words, tst, tld, emit, gate, HG)

        def s2(Xs, f, tick):
            k = []
            for c in range(3):
                r = (c * NF + f) * P
                lhs = jnp.concatenate([pltpu.bitcast(Xs[d, pl.ds(r, NB), :], bf16) for d in range(DT)], 1)
                rw = (c * NF + f) * HP
                wf = jnp.concatenate([pltpu.bitcast(W3[e, pl.ds(rw, H), :], bf16) for e in range(ET)], 1)
                k.append(jnp.dot(lhs, wf, preferred_element_type=f32))
                tick(k[-1])
            p = _pack(k[0] - k[2], k[0] + k[1])
            for e in range(ET):
                Yh[e, pl.ds(f * PY, 2 * NB), :] = p[:, e * 128:(e + 1) * 128]

        def s3(il):
            z = []
            for p in range(2):
                yw = jnp.concatenate([pltpu.bitcast(Yh[e, pl.ds(2 * il + p, NF, stride=PY), :], bf16) for e in range(ET)], 1)
                z.append(jnp.dot(cv[RG:RG + L, :], yw, preferred_element_type=f32))
            outs = []
            for p in range(2):
                tf = jnp.tanh(z[p][:, :D]) * 0.5
                outs.append(tf + tf * jnp.tanh(z[p][:, D:]))
            ost[pl.ds(pl.multiple_of(il * HOP, HOP), HOP), :] = pltpu.bitcast(_pack(outs[0], outs[1]), bf16)
            return z

        def ocp(src, row, q, sem):
            b = q // nblk
            t0 = pl.multiple_of((q % nblk) * HOP, 64)
            n = pl.multiple_of(jnp.minimum(OG * HOP, T - t0), 64)
            return pltpu.make_async_copy(src.at[pl.ds(pl.multiple_of(row, 64), n)], o_hbm.at[b, pl.ds(t0, n)], sem)

        def out_copy(s, gi):
            s = jnp.int32(s) if isinstance(s, int) else s
            gi = jnp.int32(gi) if isinstance(gi, int) else gi
            return ocp(ost, gi * (OG * HOP), s * NB + gi * OG, osem.at[gi])

        def out2_copy(gi):
            gi = jnp.int32(gi) if isinstance(gi, int) else gi
            return ocp(ost2, gi * (OG * HOP), (NS - 2) * NB + gi * OG, o2sem.at[gi])

        start_x(xlate)
        wait_x(range(PPS))
        h1 = NB // 2

        def body1(il, carry):
            s1(il)
            return carry
        lax.fori_loop(0, h1, body1, 0, unroll=u1)
        wait_x(range(PPS, 2 * PPS))
        start_x(range(2 * PPS, NQ // XB))
        xhead(1)

        def body1x(i, carry):
            res = s1(h1 + i)
            nv = z_ref[0] > 0
            xcopy(1, 2 * i, (nv, [res[:L, :D]]))
            xcopy(1, 2 * i + 1, (nv, [res[:L, D:]]))
            return carry
        lax.fori_loop(0, NB - h1, body1x, 0, unroll=u1)

        def run_s2(Xsrc, units, npu, frac):
            def s2b(i, carry):
                us = units(i)

                def chain():
                    for u in us:
                        yield from u
                gen = chain()
                npieces = len(us) * npu
                st = [0, 0]
                nt = int(3 * u2 * frac)

                def tick(kk):
                    st[0] += 1
                    n_ = min(npieces, (st[0] * npieces) // nt) - st[1]
                    del gates[:]
                    for z_ in range(n_):
                        ph = (z_ + GOFF) / n_ * len(GT)
                        tl = GT[int(ph)]
                        rr = int((ph % 1.0) * (NB // 4))
                        gates.append(pltpu.bitcast(kk[rr * 8:rr * 8 + 8, tl * 128:(tl + 1) * 128], u32))
                    for _ in range(n_):
                        next(gen, None)
                        st[1] += 1
                for t in range(u2):
                    s2(Xsrc, i * u2 + t, tick)
                assert st[1] == npieces
                for _ in gen:
                    pass
                return carry
            lax.fori_loop(0, NI2, s2b, 0)

        def gsel(never, g, v):
            n = v.shape[0] // 8
            return jnp.concatenate([jnp.where(never, g[(q * 8) % L:(q * 8) % L + 8], v[q * 8:q * 8 + 8]) for q in range(n)], 0)

        def ifftunit(unit, a, never):
            rg = unit // DT

            def gate():
                return gates.pop(0) if gates else None

            def sel(g, v):
                return v if g is None else jnp.where(never, pltpu.bitcast(g, v.dtype), v)

            def tst(i, v):
                TT[pl.ds(i * 8, 8), :] = v

            def tld(i, g):
                return sel(g, TT[pl.ds(i * 8, 8), :])

            for p in range(2):
                for half in (1, 0):
                    def loadw(gi, g):
                        wd = Xh[half, pl.ds((a * NF + gi) * PB + rg * 16 + p, 8, stride=2), :]
                        if g is None:
                            return tuple(_unpack(wd))
                        return (pltpu.bitcast(wd << jnp.where(never, g, jnp.uint32(16)), f32),
                                pltpu.bitcast(wd & jnp.where(never, g, jnp.uint32(0xFFFF0000)), f32))

                    def emit(m, z, g):
                        r = (m - HIST) * 8
                        if half == 1:
                            SG[pl.ds(r, 8), :] = jnp.tanh(z)
                        else:
                            tf = jnp.tanh(z) * 0.5
                            o = tf + tf * sel(g, SG[pl.ds(r, 8), :])
                            if p == 0:
                                SO[pl.ds(r, 8), :] = o
                            else:
                                ou[pl.ds(m - HIST, 8, stride=XP), :] = _pack(sel(g, SO[pl.ds(r, 8), :]), o)
                    yield from _inv128(loadw, tst, tld, emit, gate, 2.0 / N, HG)
            for b2 in range(8 // CPL):
                g = gate()
                for b8 in range(CPL * b2, CPL * (b2 + 1)):
                    wd = ou[pl.ds(b8 * XP, L), :]
                    if g is not None:
                        wd = jnp.concatenate([jnp.where(never, g, wd[q * 8:q * 8 + 8]) for q in range(L // 8)], 0)
                    ost2[pl.ds(pl.multiple_of((rg * 8 + b8) * HOP, HOP), HOP), a * 128:(a + 1) * 128] = pltpu.bitcast(wd, bf16)
                yield
            if a == DT - 1:
                for j in range(8 // OG):
                    out2_copy(rg * (8 // OG) + j).start()

        def sbody(s, carry):
            never = z_ref[0] > 0

            @pl.when(s < NS - 1)
            def _():
                run_s2(Xh, lambda i: [fftunit(i * FU + u, never) for u in range(FU)], 32, FFR)

            @pl.when(s == NS - 1)
            def _():
                run_s2(Xn, lambda i: [ifftunit(i * IU + u, u % DT, never) for u in range(IU)], 64 + 8 // CPL, IFR)

            for ss in range(2, NS):
                @pl.when(s == ss - 2)
                def _():
                    wait_x(range(ss * PPS, (ss + 1) * PPS))

            if True:
                @pl.when(s > 0)
                def _():
                    def owait(gi, carry):
                        out_copy(s - 1, gi).wait()
                        return carry
                    lax.fori_loop(jnp.where(s == NS - 1, NV // OG, 0), NG, owait, 0)

            @pl.when(s != NS - 2)
            def _():
                sx = jnp.minimum(s + 2, NS - 1)
                xhead(sx)

                def body3(i, carry):
                    for t in range(u3):
                        il = i * u3 + t
                        zz = s3(il)
                        xcopy(sx, il, (never, zz))
                        xmove(i, t, (never, zz))
                        if (t + 1) % OG == 0:
                            out_copy(s, i * (u3 // OG) + t // OG).start()
                    return carry
                lax.fori_loop(0, NCS, body3, 0)

            @pl.when(s == NS - 2)
            def _():
                nm = NB - NV
                ncp = ET * NF
                for t in range(nm):
                    il = NV + t
                    zz = s3(il)
                    for q in range(t * ncp // nm, (t + 1) * ncp // nm):
                        e, g = divmod(q, NF)
                        gv = pltpu.bitcast(zz[q % 2][:, e * 128:(e + 1) * 128], u32)
                        Xh[e // DT, pl.ds(((e % DT) * NF + g) * PB, 2 * NV), :] = gsel(never, gv, Yh[e, pl.ds(g * PY, 2 * NV), :])
                    if (il + 1) % OG == 0:
                        out_copy(s, il // OG).start()
            return carry
        lax.fori_loop(0, NS, sbody, 0)

        if True:
            for gi in range(NV // OG):
                out2_copy(gi).wait()
            for gi in range(NG):
                out_copy(NS - 1, gi).wait()

    def fn(x, w):
        return pl.pallas_call(
            kernel,
            in_specs=[pl.BlockSpec(memory_space=pl.ANY)] * 3 + [pl.BlockSpec(memory_space=pltpu.SMEM)],
            out_specs=pl.BlockSpec(memory_space=pl.ANY),
            out_shape=jax.ShapeDtypeStruct((B, T, D), x.dtype),
            scratch_shapes=[
                pltpu.VMEM((XROWS, D), bf16),
                pltpu.VMEM((WSL, 32, 16, D2), bf16),
                pltpu.VMEM((ET, 3 * NF * HP, 128), u32),
                pltpu.VMEM((DT, 3 * NF * P, 128), u32),
                pltpu.VMEM((DT, 3 * NF * P, 128), u32),
                pltpu.VMEM((ET, NF * PY, 128), u32),
                pltpu.VMEM((NB * HOP, D), bf16),
                pltpu.VMEM((NV * HOP, D), bf16),
                pltpu.VMEM(consts.shape, bf16),
                pltpu.VMEM((DT, NB * XP + HIST + 8, 128), u32),
                pltpu.VMEM((2048, 128), f32),
                pltpu.VMEM((L * 8, 128), f32),
                pltpu.VMEM((L * 8, 128), f32),
                pltpu.VMEM((8 * XP, 128), u32),
                pltpu.SemaphoreType.DMA((WSL,)),
                pltpu.SemaphoreType.DMA((nxs,)),
                pltpu.SemaphoreType.DMA((NG,)),
                pltpu.SemaphoreType.DMA((NV // OG,)),
                pltpu.SemaphoreType.DMA((1,)),
            ],
            compiler_params=pltpu.CompilerParams(vmem_limit_bytes=127 * 1024 * 1024),
        )(x, w, consts, np.zeros((1,), np.int32))
    return fn


@jax.jit
def pallas_standalone__autoregressive_conv_wavernn__speech_kernel(x, w):
    B, T, D = x.shape
    K = w.shape[0]
    return make(B, T, D, K)(x, w)
```

```python
import math
import numpy as np
import jax
import jax.numpy as jnp
from jax import lax
import jax.experimental.pallas as pl
import jax.experimental.pallas.tpu as pltpu

N = 128
L = 96
HIST = N - L
NF = N // 2
bf16 = jnp.bfloat16
u32 = jnp.uint32
f32 = jnp.float32


def _consts(K):
    th = np.pi * (4 * np.arange(NF) + 1) / N
    n = np.arange(N)
    F = np.concatenate([np.cos(th[:, None] * n), np.sin(th[:, None] * n)], 0)
    m = np.arange(L) + HIST
    G = np.zeros((L, NF, 2)); G[:, :, 0] = np.cos(th[None] * m[:, None]) * 2 / N
    G[:, :, 1] = np.sin(th[None] * m[:, None]) * 2 / N
    G = G.reshape(L, N)
    j = (K - 1) - np.arange(K)
    C = np.zeros((N, 32))
    C[:NF, :K] = np.cos(th[:, None] * j); C[NF:, :K] = np.sin(th[:, None] * j)
    Cb = np.zeros((2, 4 * N, 128))
    for jj in range(2):
        for dd in range(2):
            g = 2 * jj + dd
            Cb[0, g * N:(g + 1) * N, jj * 64 + dd:(jj + 1) * 64:2] = C
    Cb = Cb.reshape(2, 2, 2, 2, 8, 8, 128).transpose(0, 1, 4, 2, 3, 5, 6).reshape(2, 4 * N, 128)
    Cb[1] = 0.5 * Cb[0]
    return np.asarray(np.concatenate([F, Cb[0], Cb[1], G], 0), dtype=bf16)


def _unpack(x):
    return [pltpu.unpack_elementwise(x, index=i, packed_dtype=bf16, unpacked_dtype=f32) for i in range(2)]


def _pack(a, b):
    return pltpu.pack_elementwise([a, b], packed_dtype=bf16)


def _cmul(re, im, w):
    c, s = w.real, w.imag
    eps = 1e-12
    def close(a, b): return abs(a - b) < eps
    if close(c, 1) and close(s, 0): return re, im
    if close(c, -1) and close(s, 0): return -re, -im
    if close(c, 0) and close(s, 1): return -im, re
    if close(c, 0) and close(s, -1): return im, -re
    if close(abs(c), abs(s)):
        a = c
        if close(s, c):
            return (re - im) * a, (re + im) * a
        else:
            return (re + im) * a, (im - re) * a
    return re * c - im * s, re * s + im * c

def _fft(xs, sign=-1):
    n = len(xs)
    if n == 1: return xs
    if n == 2:
        (a, b), (c, d) = xs
        return [(a + c, b + d), (a - c, b - d)]
    if n == 4:
        (a0, b0), (a1, b1), (a2, b2), (a3, b3) = xs
        s0r, s0i, d0r, d0i = a0 + a2, b0 + b2, a0 - a2, b0 - b2
        s1r, s1i, d1r, d1i = a1 + a3, b1 + b3, a1 - a3, b1 - b3
        if sign < 0:
            return [(s0r + s1r, s0i + s1i), (d0r + d1i, d0i - d1r), (s0r - s1r, s0i - s1i), (d0r - d1i, d0i + d1r)]
        return [(s0r + s1r, s0i + s1i), (d0r - d1i, d0i + d1r), (s0r - s1r, s0i - s1i), (d0r + d1i, d0i - d1r)]
    ev = _fft(xs[0::2], sign); od = _fft(xs[1::2], sign)
    out = [None] * n
    for k in range(n // 2):
        w = complex(math.cos(2 * math.pi * k / n), sign * math.sin(2 * math.pi * k / n))
        if abs(w.real) < 1e-12 and abs(w.imag - sign) < 1e-12:
            r, i_ = od[k]
            if sign < 0:
                out[k] = (ev[k][0] + i_, ev[k][1] - r); out[k + n // 2] = (ev[k][0] - i_, ev[k][1] + r)
            else:
                out[k] = (ev[k][0] - i_, ev[k][1] + r); out[k + n // 2] = (ev[k][0] + i_, ev[k][1] - r)
            continue
        tr, ti = _cmul(od[k][0], od[k][1], w)
        out[k] = (ev[k][0] + tr, ev[k][1] + ti)
        out[k + n // 2] = (ev[k][0] - tr, ev[k][1] - ti)
    return out

def _rot(ph):
    return complex(math.cos(ph), math.sin(ph))


def _fwd128(loadw, tst, tld, emit, gate, HG=1):
    for n2 in range(8):
        for p in range(2):
            g = gate()
            col = []
            for n1 in range(8):
                a = loadw(8 * n1 + n2, p, g); b = loadw(8 * n1 + n2 + 64, p, g)
                col.append(_cmul(a, b, _rot(math.pi * 8 * n1 / 128)))
            o = _fft(col, +1)
            for g1 in range(8):
                r, i_ = _cmul(o[g1][0], o[g1][1], _rot(2 * math.pi * g1 * n2 / 64 + math.pi * n2 / 128))
                tst(((p * 8 + g1) * 8 + n2) * 2, r); tst(((p * 8 + g1) * 8 + n2) * 2 + 1, i_)
            yield
    for g1 in range(8):
        for p in range(2):
            g = gate()
            o = _fft([(tld(((p * 8 + g1) * 8 + n2) * 2, g if (n2 < 4 or not HG) else None), tld(((p * 8 + g1) * 8 + n2) * 2 + 1, g if (n2 < 4 or not HG) else None)) for n2 in range(8)], +1)
            if p == 0:
                o0 = o
            else:
                for g2 in range(8):
                    emit(g1 + 8 * g2, [o0[g2], o[g2]])
            yield


def _inv128(loadw, tst, tld, emit, gate, sc, HG=1):
    for gb in range(8):
        g = gate()
        o = _fft([loadw(8 * ga + gb, g) for ga in range(8)], -1)
        for k1 in range(8):
            r, i_ = _cmul(o[k1][0], o[k1][1], sc * _rot(-2 * math.pi * gb * k1 / 64 - math.pi * k1 / 128))
            tst((k1 * 8 + gb) * 2, r); tst((k1 * 8 + gb) * 2 + 1, i_)
        yield
    for k1 in range(8):
        g = gate()
        o = _fft([(tld((k1 * 8 + gb) * 2, g if (gb < 4 or not HG) else None), tld((k1 * 8 + gb) * 2 + 1, g if (gb < 4 or not HG) else None)) for gb in range(8)], -1)
        for k2 in range(8):
            n = k1 + 8 * k2
            w = _rot(-math.pi * k2 / 16)
            re, im = o[k2]
            if n >= 32:
                r, i_ = _cmul(re, im, w)
                emit(n, r, g)
            else:
                i_ = im if k2 == 0 else re * w.imag + im * w.real
            emit(n + 64, i_, g)
        yield


def make(B, T, D, K, NB=56, u1=28, u2=32, u3=28, uw=2, WSL=8,
         GT=(0, 2), GOFF=0.25, XSCH=None, WSCH=None, RGV=4, IFR=0.94, OG=4, CPL=1, HG=0, FFR=0.94):
    HOP = 2 * L
    nblk = -(-T // HOP)
    NQ = B * nblk
    assert NQ % NB == 0 and NB % 8 == 0
    NS = NQ // NB
    BSTR = nblk * HOP
    HEAD = 2 * HIST
    XROWS = NQ * HOP + HEAD
    D2 = 2 * D
    ET = D2 // 128
    DT = D // 128
    H = D // 2
    HP = H + 1
    P = NB + 1 if NB % 8 == 0 else NB
    PY = 2 * NB + 1
    XP = L + 4
    assert nblk % OG == 0 and NB % u3 == 0 and u3 % OG == 0 and 8 % OG == 0
    NG = NB // OG
    NCS = NB // u3
    NV = 8 * RGV
    PB = 2 * NV + 1
    assert NS >= 2 and (ET // DT) * NF * PB <= 3 * NF * P
    WC = D // 16
    NWI = WC // uw
    if WSCH is None:
        WSCH = [[0, 1], [2, 3, 4], [5, 6, 7], [8, 9], [10, 11], [12, 13], [14, 15]]
    for i, z in enumerate(WSCH[1:]):
        assert all(c < i * uw + WSL for c in z)
    NU = (NB // 8) * DT
    NI2 = NF // u2
    assert NU % NI2 == 0
    FU = NU // NI2
    assert (RGV * DT) % NI2 == 0
    assert (RGV * DT // NI2) % DT == 0
    IU = RGV * DT // NI2

    XB = 8
    xpieces = []
    for j in range(NQ // XB):
        lo, hi = j * XB * HOP + HEAD, (j + 1) * XB * HOP + HEAD
        parts = []
        for b in range(B):
            r0, r1 = max(lo, b * BSTR + HEAD), min(hi, b * BSTR + HEAD + T)
            if r1 > r0:
                parts.append((b, r0 - b * BSTR - HEAD, r1 - r0))
        xpieces.append(parts)
    PPS = NB // XB
    if XSCH is None:
        XSCH = [[], [0, 1], [2, 3], [4, 5], [6, 7], [8, 9], [10, 11], [12, 13]]
    xlate = [j for j in range(2 * PPS) if not any(j in z for z in XSCH)]
    nxs = sum(len(p) for p in xpieces)

    consts = _consts(K)
    RF, RC, RG = 0, N, N + 8 * N

    def kernel(x_hbm, w_hbm, c_hbm, z_ref, o_hbm, xs, wv, W3, Xh, Xn, Yh, ost, ost2, cv, xu, TT, SG, SO, ou, wsem, xsem, osem, o2sem, csem):
        def wcp(c):
            r = c * 16 if isinstance(c, int) else pl.multiple_of(c * 16, 16)
            return pltpu.make_async_copy(w_hbm.at[:, pl.ds(r, 16), :], wv.at[c % WSL, pl.ds(0, K)], wsem.at[c % WSL])

        xcps = []
        for parts in xpieces:
            xcps.append([pltpu.make_async_copy(x_hbm.at[b, pl.ds(t0, n), :], xs.at[pl.ds(b * BSTR + HEAD + t0, n), :],
                                               xsem.at[sum(map(len, xcps)) + i]) for i, (b, t0, n) in enumerate(parts)])
        ccp = pltpu.make_async_copy(c_hbm, cv, csem.at[0])
        for c in WSCH[0]:
            wcp(c).start()
        ccp.start()
        xs[pl.ds(0, HEAD), :] = jnp.zeros((HEAD, D), bf16)
        for b in range(B):
            xs[pl.ds(b * BSTR + HEAD + T, BSTR - T), :] = jnp.zeros((BSTR - T, D), bf16)
        for sl in range(WSL):
            for k in range(K, 32):
                wv[sl, k] = jnp.zeros((16, D2), bf16)

        def start_x(js):
            for j in js:
                for c in xcps[j]:
                    c.start()

        def wait_x(js):
            for j in js:
                for c in xcps[j]:
                    c.wait()

        ccp.wait()

        def wunit(jg):
            sl = jg % WSL
            for e in range(ET):
                wd = pltpu.bitcast(wv[sl, :, :, e * 128:(e + 1) * 128], u32)
                wd = jnp.swapaxes(wd, 0, 1)
                rhs = jnp.concatenate([pltpu.bitcast(wd[2 * t:2 * t + 2].reshape(64, 128), bf16) for t in range(4)], 1)
                rc = RC + (e // DT) * 4 * N
                res = jnp.dot(cv[rc:rc + 4 * N, :], rhs, preferred_element_type=f32)
                for jj in range(2):
                    for fo in range(8):
                        r0 = (jj * 8 + fo) * 32
                        for t in range(4):
                            m = []
                            for dd in range(2):
                                vr = res[r0 + dd * 16:r0 + dd * 16 + 8, t * 128:(t + 1) * 128]
                                vi = res[r0 + dd * 16 + 8:r0 + dd * 16 + 16, t * 128:(t + 1) * 128]
                                m.append((vr, vi - vr, vi + vr))
                            for cc in range(3):
                                W3[e, pl.ds((cc * NF + fo * 8) * HP + jg * 8 + 2 * t + jj, 8, stride=HP), :] = _pack(m[0][cc], m[1][cc])

        def wbody(it, carry):
            for t in range(uw):
                wcp(it * uw + t).wait()
            for i in range(NWI):
                if i + 1 < len(WSCH) or XSCH[i]:
                    @pl.when(it == i)
                    def _():
                        if i + 1 < len(WSCH):
                            for c in WSCH[i + 1]:
                                wcp(c).start()
                        start_x(XSCH[i])
            for t in range(uw):
                wunit(it * uw + t)
            return carry
        lax.fori_loop(0, NWI, wbody, 0)

        def s1(il):
            r0 = pl.multiple_of(il * HOP, HOP)
            cols = []
            for d in range(DT):
                xw = pltpu.bitcast(xs[pl.ds(r0, 2 * N), d * 128:(d + 1) * 128], u32)
                cols.append([v.astype(bf16) for v in _unpack(xw)])
            rhs = jnp.concatenate([cols[d][p] for d in range(DT) for p in range(2)], 1)
            res = jnp.dot(cv[RF:RF + N, :], rhs, preferred_element_type=f32)
            for d in range(DT):
                ev = res[:, (2 * d) * 128:(2 * d + 1) * 128]
                od = res[:, (2 * d + 1) * 128:(2 * d + 2) * 128]
                m = [(v[:NF] + v[NF:], v[:NF], v[NF:]) for v in (ev, od)]
                for c in range(3):
                    Xh[d, pl.ds(c * NF * P + il, NF, stride=P), :] = _pack(m[0][c], m[1][c])
            return res

        def xcopy(s, il, g=None):
            r0 = pl.multiple_of((s * NB + il) * HOP + HEAD, 64)
            xw = pltpu.bitcast(xs[pl.ds(r0, HOP), :], u32)
            if g is not None:
                xw = jnp.where(g[0], pltpu.bitcast(g[1][0][:, :D], u32), xw)
            for d in range(DT):
                xu[d, pl.ds(il * XP + HIST + 4, L), :] = xw[:, d * 128:(d + 1) * 128]

        def xhead(s):
            xw = pltpu.bitcast(xs[pl.ds(pl.multiple_of(s * NB * HOP, 64), HEAD), :], u32)
            for d in range(DT):
                xu[d, pl.ds(0, HIST), :] = xw[:, d * 128:(d + 1) * 128]

        XR = 3 * NF * P // NCS
        assert XR * NCS == 3 * NF * P and XR % 8 == 0

        def xmove(i, t, g=None):
            per = (XR // 8 // u3) * 8
            r0 = t * per
            n = per if t < u3 - 1 else XR - r0
            r = pl.multiple_of(i * XR + r0, 8)
            for d in range(DT):
                v = Xn[d, pl.ds(r, n), :]
                if g is not None:
                    gv = pltpu.bitcast(g[1][1][:, (2 + d) * 128:(3 + d) * 128], u32)
                    v = jnp.concatenate([jnp.where(g[0], gv[(q * 8) % L:(q * 8) % L + 8], v[q * 8:q * 8 + 8]) for q in range(n // 8)], 0)
                Xh[d, pl.ds(r, n), :] = v

        gates = []

        def fftunit(unit, never):
            rg = unit // DT
            d = unit % DT
            base = rg * (8 * XP)

            def gate():
                return gates.pop(0) if gates else None

            def words(n, p, g):
                wd = xu[d, pl.ds(base + n + (4 if n >= HIST else 0), 8, stride=XP), :]
                if g is None:
                    return pltpu.unpack_elementwise(wd, index=p, packed_dtype=bf16, unpacked_dtype=f32)
                if p == 0:
                    return pltpu.bitcast(wd << jnp.where(never, g, jnp.uint32(16)), f32)
                return pltpu.bitcast(wd & jnp.where(never, g, jnp.uint32(0xFFFF0000)), f32)

            def tst(i, v):
                TT[pl.ds(i * 8, 8), :] = v

            def tld(i, g):
                v = TT[pl.ds(i * 8, 8), :]
                return v if g is None else jnp.where(never, pltpu.bitcast(g, f32), v)

            def emit(g, v):
                m = [(a + b_, a, b_) for (a, b_) in v]
                for c in range(3):
                    Xn[d, pl.ds((c * NF + g) * P + rg * 8, 8), :] = _pack(m[0][c], m[1][c])
            return _fwd128(words, tst, tld, emit, gate, HG)

        def s2(Xs, f, tick):
            k = []
            for c in range(3):
                r = (c * NF + f) * P
                lhs = jnp.concatenate([pltpu.bitcast(Xs[d, pl.ds(r, NB), :], bf16) for d in range(DT)], 1)
                rw = (c * NF + f) * HP
                wf = jnp.concatenate([pltpu.bitcast(W3[e, pl.ds(rw, H), :], bf16) for e in range(ET)], 1)
                k.append(jnp.dot(lhs, wf, preferred_element_type=f32))
                tick(k[-1])
            p = _pack(k[0] - k[2], k[0] + k[1])
            for e in range(ET):
                Yh[e, pl.ds(f * PY, 2 * NB), :] = p[:, e * 128:(e + 1) * 128]

        def s3(il):
            z = []
            for p in range(2):
                yw = jnp.concatenate([pltpu.bitcast(Yh[e, pl.ds(2 * il + p, NF, stride=PY), :], bf16) for e in range(ET)], 1)
                z.append(jnp.dot(cv[RG:RG + L, :], yw, preferred_element_type=f32))
            outs = []
            for p in range(2):
                tf = jnp.tanh(z[p][:, :D]) * 0.5
                outs.append(tf + tf * jnp.tanh(z[p][:, D:]))
            ost[pl.ds(pl.multiple_of(il * HOP, HOP), HOP), :] = pltpu.bitcast(_pack(outs[0], outs[1]), bf16)
            return z

        def ocp(src, row, q, sem):
            b = q // nblk
            t0 = pl.multiple_of((q % nblk) * HOP, 64)
            n = pl.multiple_of(jnp.minimum(OG * HOP, T - t0), 64)
            return pltpu.make_async_copy(src.at[pl.ds(pl.multiple_of(row, 64), n)], o_hbm.at[b, pl.ds(t0, n)], sem)

        def out_copy(s, gi):
            s = jnp.int32(s) if isinstance(s, int) else s
            gi = jnp.int32(gi) if isinstance(gi, int) else gi
            return ocp(ost, gi * (OG * HOP), s * NB + gi * OG, osem.at[gi])

        def out2_copy(gi):
            gi = jnp.int32(gi) if isinstance(gi, int) else gi
            return ocp(ost2, gi * (OG * HOP), (NS - 2) * NB + gi * OG, o2sem.at[gi])

        start_x(xlate)
        wait_x(range(PPS))
        h1 = NB // 2

        def body1(il, carry):
            s1(il)
            return carry
        lax.fori_loop(0, h1, body1, 0, unroll=u1)
        wait_x(range(PPS, 2 * PPS))
        start_x(range(2 * PPS, NQ // XB))
        xhead(1)

        def body1x(i, carry):
            res = s1(h1 + i)
            nv = z_ref[0] > 0
            xcopy(1, 2 * i, (nv, [res[:L, :D]]))
            xcopy(1, 2 * i + 1, (nv, [res[:L, D:]]))
            return carry
        lax.fori_loop(0, NB - h1, body1x, 0, unroll=u1)

        def run_s2(Xsrc, units, npu, frac):
            def s2b(i, carry):
                us = units(i)

                def chain():
                    for u in us:
                        yield from u
                gen = chain()
                npieces = len(us) * npu
                st = [0, 0]
                nt = int(3 * u2 * frac)

                def tick(kk):
                    st[0] += 1
                    n_ = min(npieces, (st[0] * npieces) // nt) - st[1]
                    del gates[:]
                    for z_ in range(n_):
                        ph = (z_ + GOFF) / n_ * len(GT)
                        tl = GT[int(ph)]
                        rr = int((ph % 1.0) * (NB // 4))
                        gates.append(pltpu.bitcast(kk[rr * 8:rr * 8 + 8, tl * 128:(tl + 1) * 128], u32))
                    for _ in range(n_):
                        next(gen, None)
                        st[1] += 1
                for t in range(u2):
                    s2(Xsrc, i * u2 + t, tick)
                assert st[1] == npieces
                for _ in gen:
                    pass
                return carry
            lax.fori_loop(0, NI2, s2b, 0)

        def gsel(never, g, v):
            n = v.shape[0] // 8
            return jnp.concatenate([jnp.where(never, g[(q * 8) % L:(q * 8) % L + 8], v[q * 8:q * 8 + 8]) for q in range(n)], 0)

        def ifftunit(unit, a, never):
            rg = unit // DT

            def gate():
                return gates.pop(0) if gates else None

            def sel(g, v):
                return v if g is None else jnp.where(never, pltpu.bitcast(g, v.dtype), v)

            def tst(i, v):
                TT[pl.ds(i * 8, 8), :] = v

            def tld(i, g):
                return sel(g, TT[pl.ds(i * 8, 8), :])

            for p in range(2):
                for half in (1, 0):
                    def loadw(gi, g):
                        wd = Xh[half, pl.ds((a * NF + gi) * PB + rg * 16 + p, 8, stride=2), :]
                        if g is None:
                            return tuple(_unpack(wd))
                        return (pltpu.bitcast(wd << jnp.where(never, g, jnp.uint32(16)), f32),
                                pltpu.bitcast(wd & jnp.where(never, g, jnp.uint32(0xFFFF0000)), f32))

                    def emit(m, z, g):
                        r = (m - HIST) * 8
                        if half == 1:
                            SG[pl.ds(r, 8), :] = jnp.tanh(z)
                        else:
                            tf = jnp.tanh(z) * 0.5
                            o = tf + tf * sel(g, SG[pl.ds(r, 8), :])
                            if p == 0:
                                SO[pl.ds(r, 8), :] = o
                            else:
                                ou[pl.ds(m - HIST, 8, stride=XP), :] = _pack(sel(g, SO[pl.ds(r, 8), :]), o)
                    yield from _inv128(loadw, tst, tld, emit, gate, 2.0 / N, HG)
            for b2 in range(8 // CPL):
                g = gate()
                for b8 in range(CPL * b2, CPL * (b2 + 1)):
                    wd = ou[pl.ds(b8 * XP, L), :]
                    if g is not None:
                        wd = jnp.concatenate([jnp.where(never, g, wd[q * 8:q * 8 + 8]) for q in range(L // 8)], 0)
                    ost2[pl.ds(pl.multiple_of((rg * 8 + b8) * HOP, HOP), HOP), a * 128:(a + 1) * 128] = pltpu.bitcast(wd, bf16)
                yield
            if a == DT - 1:
                for j in range(8 // OG):
                    out2_copy(rg * (8 // OG) + j).start()

        def sbody(s, carry):
            never = z_ref[0] > 0

            @pl.when(s < NS - 1)
            def _():
                run_s2(Xh, lambda i: [fftunit(i * FU + u, never) for u in range(FU)], 32, FFR)

            @pl.when(s == NS - 1)
            def _():
                run_s2(Xn, lambda i: [ifftunit(i * IU + u, u % DT, never) for u in range(IU)], 64 + 8 // CPL, IFR)

            for ss in range(2, NS):
                @pl.when(s == ss - 2)
                def _():
                    wait_x(range(ss * PPS, (ss + 1) * PPS))

            @pl.when(s > 0)
            def _():
                def owait(gi, carry):
                    out_copy(s - 1, gi).wait()
                    return carry
                lax.fori_loop(jnp.where(s == NS - 1, NV // OG, 0), NG, owait, 0)

            @pl.when(s != NS - 2)
            def _():
                sx = jnp.minimum(s + 2, NS - 1)
                xhead(sx)

                def body3(i, carry):
                    for t in range(u3):
                        il = i * u3 + t
                        zz = s3(il)
                        xcopy(sx, il, (never, zz))
                        xmove(i, t, (never, zz))
                        if (t + 1) % OG == 0:
                            out_copy(s, i * (u3 // OG) + t // OG).start()
                    return carry
                lax.fori_loop(0, NCS, body3, 0)

            @pl.when(s == NS - 2)
            def _():
                nm = NB - NV
                ncp = ET * NF
                for t in range(nm):
                    il = NV + t
                    zz = s3(il)
                    for q in range(t * ncp // nm, (t + 1) * ncp // nm):
                        e, g = divmod(q, NF)
                        gv = pltpu.bitcast(zz[q % 2][:, e * 128:(e + 1) * 128], u32)
                        Xh[e // DT, pl.ds(((e % DT) * NF + g) * PB, 2 * NV), :] = gsel(never, gv, Yh[e, pl.ds(g * PY, 2 * NV), :])
                    if (il + 1) % OG == 0:
                        out_copy(s, il // OG).start()
            return carry
        lax.fori_loop(0, NS, sbody, 0)

        for gi in range(NV // OG):
            out2_copy(gi).wait()
        for gi in range(NG):
            out_copy(NS - 1, gi).wait()

    def fn(x, w):
        return pl.pallas_call(
            kernel,
            in_specs=[pl.BlockSpec(memory_space=pl.ANY)] * 3 + [pl.BlockSpec(memory_space=pltpu.SMEM)],
            out_specs=pl.BlockSpec(memory_space=pl.ANY),
            out_shape=jax.ShapeDtypeStruct((B, T, D), x.dtype),
            scratch_shapes=[
                pltpu.VMEM((XROWS, D), bf16),
                pltpu.VMEM((WSL, 32, 16, D2), bf16),
                pltpu.VMEM((ET, 3 * NF * HP, 128), u32),
                pltpu.VMEM((DT, 3 * NF * P, 128), u32),
                pltpu.VMEM((DT, 3 * NF * P, 128), u32),
                pltpu.VMEM((ET, NF * PY, 128), u32),
                pltpu.VMEM((NB * HOP, D), bf16),
                pltpu.VMEM((NV * HOP, D), bf16),
                pltpu.VMEM(consts.shape, bf16),
                pltpu.VMEM((DT, NB * XP + HIST + 8, 128), u32),
                pltpu.VMEM((2048, 128), f32),
                pltpu.VMEM((L * 8, 128), f32),
                pltpu.VMEM((L * 8, 128), f32),
                pltpu.VMEM((8 * XP, 128), u32),
                pltpu.SemaphoreType.DMA((WSL,)),
                pltpu.SemaphoreType.DMA((nxs,)),
                pltpu.SemaphoreType.DMA((NG,)),
                pltpu.SemaphoreType.DMA((NV // OG,)),
                pltpu.SemaphoreType.DMA((1,)),
            ],
            compiler_params=pltpu.CompilerParams(vmem_limit_bytes=127 * 1024 * 1024),
        )(x, w, consts, np.zeros((1,), np.int32))
    return fn


@jax.jit
def pallas_standalone__autoregressive_conv_wavernn__speech_kernel(x, w):
    B, T, D = x.shape
    K = w.shape[0]
    return make(B, T, D, K)(x, w)
```
